```python
import os as _os
_os.environ.setdefault("JAX_PLATFORMS", "cpu")
import jax
import jax.numpy as jnp

def _softmax(x, axis=-1):
    return jax.nn.softmax(x, axis=axis)
def _gelu(x):
    return jax.nn.gelu(x, approximate=True)
def _silu(x):
    return jax.nn.silu(x)
def _sigmoid(x):
    return jax.nn.sigmoid(x)
def _layernorm(x, axis=-1, eps=1e-5):
    m = jnp.mean(x, axis=axis, keepdims=True)
    v = jnp.var(x, axis=axis, keepdims=True)
    return (x - m) / jnp.sqrt(v + eps)
def _scatter_add(tgt, idx, src, axis=0):
    return tgt.at[idx].add(src)
def _segment_sum(src, seg, n):
    return jax.ops.segment_sum(src, seg, n)
class _Rng:
    def __init__(self, key):
        self._k = key
    def _next(self):
        self._k, sub = jax.random.split(self._k)
        return sub
    def normal(self, shape):
        return jax.random.normal(self._next(), shape, dtype=jnp.bfloat16)
    def randint(self, lo, hi, shape):
        return jax.random.randint(self._next(), shape, lo, hi, dtype=jnp.int32)
    def uniform(self, shape, lo=0.0, hi=1.0):
        return jax.random.uniform(self._next(), shape, jnp.bfloat16, lo, hi)
    def permutation(self, n):
        return jax.random.permutation(self._next(), n)


kernel_name = 'concat_heads__softmax_full_mha__grouped_kv_mqa__prompt'

def setup_inputs():
    _rng = _Rng(jax.random.key(int.from_bytes(__import__("os").urandom(4), "little")))
    _w = (lambda a: (lambda t: t.astype(jnp.bfloat16) if jnp.issubdtype(t.dtype, jnp.floating) else t)(jnp.asarray(a)))
    def _A_setup():
        B, S, D = 1, 2048, 640
        return {
            "x": _w((lambda *s: _rng.normal(s) * 0.1)(B, S, D)),
            "wqkv": _w((lambda *s: _rng.normal(s) * 0.1)(D, 3 * D)),
            "wo": _w((lambda *s: _rng.normal(s) * 0.05)(D, D)),
        }
    _A_in = _A_setup()

    def _B_setup():
        B, S, D, H = 1, 2048, 640, 32
        Dh = D // H
        return {
            "x": _w((lambda *s: _rng.normal(s) * 0.05)(B, S, D)),
            "wq": _w((lambda *s: _rng.normal(s) * 0.4)(D, H * Dh)),
            "wk": _w((lambda *s: _rng.normal(s) * 0.4)(D, Dh)),
            "wv": _w((lambda *s: _rng.normal(s) * 0.05)(D, Dh)),
            "wo": _w((lambda *s: _rng.normal(s) * 0.05)(H * Dh, D)),
        }
    _B_in = _B_setup()

    return {
        "A_x": _A_in["x"],
        "A_wqkv": _A_in["wqkv"],
        "A_wo": _A_in["wo"],
        "B_x": _B_in["x"],
        "B_wq": _B_in["wq"],
        "B_wk": _B_in["wk"],
        "B_wv": _B_in["wv"],
        "B_wo": _B_in["wo"],
    }

def reference(A_x, A_wqkv, A_wo, B_x, B_wq, B_wk, B_wv, B_wo):
    def _A_ref(x, wqkv, wo):
        B, S, D = x.shape
        H = 32; Dh = D // H
        qkv = (lambda x, *d: x.transpose(*d))((x @ wqkv).reshape(B, S, 3, H, Dh), 2, 0, 3, 1, 4)
        q, k, v = qkv[0], qkv[1], qkv[2]
        scale = Dh ** -0.5
        scores = jnp.einsum("bhqd,bhkd->bhqk", q, k) * scale
        p = _softmax(scores, axis=-1)
        o = jnp.einsum("bhqk,bhkd->bhqd", p, v)
        return (lambda x, *d: x.transpose(*d))(o, 0, 2, 1, 3).reshape(B, S, D) @ wo

    def _B_ref(x, wq, wk, wv, wo):
        B, S, D = x.shape
        H = 32
        Dh = D // H
        q = (lambda x, *d: x.transpose(*d))((x @ wq).reshape(B, S, H, Dh), 0, 2, 1, 3)
        k = x @ wk
        v = x @ wv
        scores = jnp.einsum("bhqd,bkd->bhqk", q, k) * (Dh ** -0.5)
        p = _softmax(scores, axis=-1)
        o = jnp.einsum("bhqk,bkd->bhqd", p, v)
        return (lambda x, *d: x.transpose(*d))(o, 0, 2, 1, 3).reshape(B, S, H * Dh) @ wo

    a = _A_ref(A_x, A_wqkv, A_wo)
    b = _B_ref(B_x, B_wq, B_wk, B_wv, B_wo)
    return jnp.concatenate([a, b], axis=-1)
```

```python
import functools
import math

import jax
import jax.numpy as jnp
from jax import lax
import jax.experimental.pallas as pl
import jax.experimental.pallas.tpu as pltpu

S = 2048
D = 640
H = 32
DH = 20
HPG = 6
NG = 6
DV = 24
QB = 256
KC = 256
NQ = S // QB
NK = S // KC
PB = 512
QSCALE = (DH ** -0.5) * math.log2(math.e)


def _kernel(xa_ref, wta_ref, wka_ref, woa_ref, xb_ref, wtb_ref, wkb_ref, wob_ref,
            o_ref,
            qta, qtb, ka, kb, vta, vtb, ota, otb,
            s0, s1, s2, s3, m0, m1, m2, m3):
    f32 = jnp.float32
    bf16 = jnp.bfloat16
    nt = (((1,), (1,)), ((), ()))

    for r in range(S // PB):
        rows = slice(r * PB, (r + 1) * PB)
        xblk = xa_ref[rows, :]
        qv = lax.dot_general(wta_ref[...], xblk, nt, preferred_element_type=f32)
        for j in range(PB // QB):
            qta[r * (PB // QB) + j] = (qv[:NG * 128, j * QB:(j + 1) * QB] * QSCALE).reshape(NG, 128, QB)
        v = qv[NG * 128:, :].reshape(H, DV, PB)
        rid = lax.broadcasted_iota(jnp.int32, (H, DV, PB), 1)
        vta[:, :, rows] = jnp.where(rid == DH, 1.0, v)
        k = jnp.dot(xblk, wka_ref[...], preferred_element_type=f32).astype(bf16)
        for g in range(NG):
            ka[g, rows, :] = k[:, g * 128:(g + 1) * 128]

        xblk = xb_ref[rows, :]
        qv = lax.dot_general(wtb_ref[...], xblk, nt, preferred_element_type=f32)
        for j in range(PB // QB):
            qtb[r * (PB // QB) + j] = (qv[:NG * 128, j * QB:(j + 1) * QB] * QSCALE).reshape(NG, 128, QB)
        v = qv[NG * 128:NG * 128 + DV, :]
        rid = lax.broadcasted_iota(jnp.int32, (DV, PB), 0)
        vtb[:, rows] = jnp.where(rid == DH, 1.0, v)
        kb[rows, :] = jnp.dot(xblk, wkb_ref[...], preferred_element_type=f32).astype(bf16)

    def masked_q(qt, j):
        qi = j // H
        h = j % H
        g = h // HPG
        r0 = (h % HPG) * DH
        rows = lax.broadcasted_iota(jnp.int32, (128, QB), 0)
        msk = (rows >= r0) & (rows < r0 + DH)
        return jnp.where(msk, qt[qi, g], 0.0).astype(bf16), g, h

    def step(is_a, j, j1, s_cur, m_cur_ref, s_nxt, m_nxt_ref, do1=True, do2=True):
        if do1:
            qm, g1, _ = masked_q(qta if is_a else qtb, j1)
        if do2:
            h = j % H
            m_cur = m_cur_ref[...]
        mx = None
        acc = None
        for c in range(NK):
            ks = pl.ds(c * KC, KC)
            if do1:
                kblk = ka[g1, ks, :] if is_a else kb[ks, :]
                s = jnp.dot(kblk, qm, preferred_element_type=f32)
                s_nxt[ks, :] = s
                sm = jnp.max(s.reshape(KC // 8, 8, QB), axis=0)
                mx = sm if mx is None else jnp.maximum(mx, sm)
            if do2:
                p = jnp.exp2((s_cur[ks, :].reshape(KC // 8, 8, QB) - m_cur[None]).reshape(KC, QB))
                vblk = vta[h, :, ks] if is_a else vtb[:, ks]
                d = jnp.dot(vblk, p, preferred_element_type=f32)
                acc = d if acc is None else acc + d
        if do1:
            m_nxt_ref[...] = jnp.broadcast_to(jnp.max(mx, axis=0, keepdims=True), (8, QB))
        if do2:
            o = acc * (1.0 / acc[DH:DH + 1, :])
            if is_a:
                ota[h] = o
            else:
                otb[h] = o

    step(True, 0, 0, None, None, s0, m0, do2=False)
    step(False, 0, 0, None, None, s1, m1, do2=False)

    tn = (((0,), (0,)), ((), ()))

    def qblock(qi, carry):
        def body(i, carry2):
            j = qi * H + 2 * i
            step(True, j, j + 1, s0, m0, s2, m2)
            step(False, j, j + 1, s1, m1, s3, m3)
            j2 = jnp.minimum(j + 2, NQ * H - 1)
            step(True, j + 1, j2, s2, m2, s0, m0)
            step(False, j + 1, j2, s3, m3, s1, m1)
            return carry2
        lax.fori_loop(0, H // 2, body, 0)
        rows = pl.ds(pl.multiple_of(qi * QB, QB), QB)
        oa = ota[...].reshape(H * DV, QB).astype(bf16)
        o_ref[rows, 0:D] = lax.dot_general(oa, woa_ref[...], tn, preferred_element_type=f32).astype(bf16)
        ob = otb[...].reshape(H * DV, QB).astype(bf16)
        o_ref[rows, D:2 * D] = lax.dot_general(ob, wob_ref[...], tn, preferred_element_type=f32).astype(bf16)
        return carry

    lax.fori_loop(0, NQ, qblock, 0)


def _group6(w):
    w = jnp.pad(w, ((0, 0), (0, NG * HPG * DH - H * DH))).reshape(D, NG, HPG * DH)
    return jnp.pad(w, ((0, 0), (0, 0), (0, 128 - HPG * DH))).reshape(D, NG * 128)


def _pad24(w):
    return jnp.pad(w.reshape(D, H, DH), ((0, 0), (0, 0), (0, DV - DH))).reshape(D, H * DV)


def _pad24_rows(w):
    return jnp.pad(w.reshape(H, DH, D), ((0, 0), (0, DV - DH), (0, 0))).reshape(H * DV, D)


@jax.jit
def pallas_concat_heads__softmax_full_mha__grouped_kv_mqa__prompt_kernel(
    A_x, A_wqkv, A_wo, B_x, B_wq, B_wk, B_wv, B_wo):
    xa = A_x.reshape(S, D)
    xb = B_x.reshape(S, D)
    wta = jnp.concatenate([_group6(A_wqkv[:, :D]), _pad24(A_wqkv[:, 2 * D:])], axis=1).T
    wka = _group6(A_wqkv[:, D:2 * D])
    woa = _pad24_rows(A_wo)
    wtb = jnp.concatenate([_group6(B_wq), jnp.pad(B_wv, ((0, 0), (0, 32 - DH)))], axis=1).T
    wkb = jnp.pad(jnp.tile(B_wk, (1, HPG)), ((0, 0), (0, 128 - HPG * DH)))
    wob = _pad24_rows(B_wo)
    f32 = jnp.float32
    bf16 = jnp.bfloat16
    out = pl.pallas_call(
        _kernel,
        out_shape=jax.ShapeDtypeStruct((S, 2 * D), bf16),
        scratch_shapes=[
            pltpu.VMEM((NQ, NG, 128, QB), f32), pltpu.VMEM((NQ, NG, 128, QB), f32),
            pltpu.VMEM((NG, S, 128), bf16), pltpu.VMEM((S, 128), bf16),
            pltpu.VMEM((H, DV, S), f32), pltpu.VMEM((DV, S), f32),
            pltpu.VMEM((H, DV, QB), f32), pltpu.VMEM((H, DV, QB), f32),
        ] + [pltpu.VMEM((S, QB), f32)] * 4 + [pltpu.VMEM((8, QB), f32)] * 4,
        compiler_params=pltpu.CompilerParams(vmem_limit_bytes=100 * 1024 * 1024),
    )(xa, wta, wka, woa, xb, wtb, wkb, wob)
    return out.reshape(1, S, 2 * D)
```

```python
import functools
import math
import os

import jax
import jax.numpy as jnp
from jax import lax
import jax.experimental.pallas as pl
import jax.experimental.pallas.tpu as pltpu

S = 2048
D = 640
H = 32
DH = 20
QB = 512
T = QB // 128
NQ = S // QB
KC = 128
NK = S // KC
PB = 512
QSCALE = (DH ** -0.5) * math.log2(math.e)
WIN = (0, 120, 240, 360, 480, 512)
NVG = int(os.environ.get("NVG", 56))
NCH = int(os.environ.get("NCH", 4))
NV = NVG * 8
NM = S - NV
NITEMS = NQ * H

f32 = jnp.float32
bf16 = jnp.bfloat16
u32 = jnp.uint32
NT = (((1,), (1,)), ((), ()))
TN = (((0,), (0,)), ((), ()))


def _kernel(xa_h, wqkv_h, woa_h, xb_h, wq_h, wk_h, wv_h, wob_h,
            out_h,
            xa, wqkv, woa, xb, wq, wk, wv, wob,
            wta, wtb, wkw, wkb,
            qta, qtb, ka, kb, vta, vtb, ota, otb, kbc,
            sa0, sa1, sb0, sb1, ma0, ma1, mb0, mb1,
            qr0, qr1, wa0, wa1, wb0, wb1,
            obuf, tab, isem, osem):
    srcs = (wqkv_h, xa_h, wq_h, wk_h, wv_h, xb_h, woa_h, wob_h)
    dsts = (wqkv, xa, wq, wk, wv, xb, woa, wob)
    cps = [pltpu.make_async_copy(s, d, isem.at[i]) for i, (s, d) in enumerate(zip(srcs, dsts))]
    for c in cps:
        c.start()

    for h in range(H):
        g = min(h // 6, 5)
        tab[0, h] = g
        tab[1, h] = WIN[g]
        tab[2, h] = h * DH - WIN[g]

    cps[0].wait()
    wta[0:D, :] = wqkv[:, 0:D].T
    wta[D:2 * D, :] = wqkv[:, 2 * D:3 * D].T
    for g in range(6):
        wkw[:, g * 128:(g + 1) * 128] = wqkv[:, D + WIN[g]:D + WIN[g] + 128]
    cps[1].wait()
    for r in range(S // PB):
        rows = slice(r * PB, (r + 1) * PB)
        xblk = xa[rows, :]
        qv = lax.dot_general(wta[...], xblk, NT, preferred_element_type=f32)
        qta[r] = qv[:D] * QSCALE
        vta[:, :, rows] = qv[D:].reshape(H // 2, 2 * DH, PB)
        k = jnp.dot(xblk, wkw[...], preferred_element_type=f32).astype(bf16)
        for g in range(6):
            ka[g, r * PB // 2:(r + 1) * PB // 2, :] = pltpu.bitcast(k[:, g * 128:(g + 1) * 128], u32)

    for i in (2, 3, 4):
        cps[i].wait()
    wtb[0:D, :] = wq[...].T
    wkv = jnp.concatenate([wk[...], wk[...], wv[...], jnp.zeros((D, 128 - 3 * DH), bf16)], axis=1)
    wkb[...] = wkv
    wtb[D:D + 128, :] = wkv.T
    cps[5].wait()
    for r in range(S // PB):
        rows = slice(r * PB, (r + 1) * PB)
        xblk = xb[rows, :]
        qv = lax.dot_general(wtb[0:D + 64, :], xblk, NT, preferred_element_type=f32)
        q = (qv[:D] * QSCALE).astype(bf16).astype(f32)
        for l in range(PB // 128):
            qtb[r * (PB // 128) + l] = q[:, l * 128:(l + 1) * 128]
        v = qv[D + 2 * DH:D + 2 * DH + 24]
        rid = lax.broadcasted_iota(jnp.int32, (24, PB), 0)
        vtb[:, rows] = jnp.where(rid == DH, 1.0, v)
        k = jnp.dot(xblk, wkb[...], preferred_element_type=f32).astype(bf16)
        kb[r * PB // 2:(r + 1) * PB // 2, :] = pltpu.bitcast(k, u32)
    if NVG:
        er = lax.broadcasted_iota(jnp.int32, (32, DH * 128), 0)
        ec = lax.broadcasted_iota(jnp.int32, (32, DH * 128), 1)
        e = jnp.where((ec >= er * 128) & (ec < er * 128 + 128), 1.0, 0.0).astype(bf16)
        kt = pltpu.bitcast(kb[NM // 2:S // 2, :], bf16)[:, :32]
        bc = jnp.dot(kt, e, preferred_element_type=f32)
        for d in range(DH):
            kbc[d] = bc[:, d * 128:(d + 1) * 128]
    cps[6].wait()
    cps[7].wait()

    qrs = (qr0, qr1)
    was = (wa0, wa1)
    wbs = (wb0, wb1)

    def prep(j2, par2):
        qi = j2 // H
        h = j2 % H
        st = pl.multiple_of(tab[1, h], 8)
        lo = tab[2, h]
        rows = lax.broadcasted_iota(jnp.int32, (128, QB), 0)
        msk = (rows >= lo) & (rows < lo + DH)
        was[par2][...] = pltpu.bitcast(jnp.where(msk, qta[qi, pl.ds(st, 128), :], 0.0).astype(bf16), u32)
        st = pl.multiple_of((h // 2) * 2 * DH, 8)
        qq = jnp.concatenate([qtb[qi * T + l, pl.ds(st, 24 if par2 == 0 else 40), :] for l in range(T)], axis=1)
        qq = jnp.concatenate([qq, jnp.zeros((8, QB), f32)], axis=0)
        rows = lax.broadcasted_iota(jnp.int32, qq.shape, 0)
        msk = (rows < DH) if par2 == 0 else (rows >= DH)
        wbs[par2][...] = pltpu.bitcast(jnp.where(msk, qq, 0.0).astype(bf16), u32)
        if NVG:
            for d in range(DH):
                for l in range(T):
                    qrs[par2][d, :, l * 128:(l + 1) * 128] = qtb[qi * T + l, pl.ds(st + par2 * DH + d, 8, stride=0), :]

    def item(j, par, j1, sin, sout, min_, mout, do1=True, do2=True):
        par1 = 1 - par
        qk_units = []
        pv_units = []
        for c in range(NK):
            if do1:
                qk_units.append((0, c * KC, KC))
                if c * KC < NM:
                    qk_units.append((1, c * KC, min(KC, NM - c * KC)))
            if do2:
                pv_units.append((0, c))
                pv_units.append((1, c))
        qms = {}
        accs = {}
        mx = {}
        if do1:
            g1 = tab[0, j1 % H]
            never = lax.broadcasted_iota(jnp.int32, (8, 128), 0) > (j1 + 1000)
        if do2:
            hp = (j % H) // 2
        anchor = []
        vmx = [[] for _ in range(T)]
        vun = [(r, l) for l in range(T) for r in range(NVG)] if do1 else []

        def vpu_gen():
            link = [None] * NCH
            run = [(None, None)] * NCH

            def qrow(l, d):
                return qrs[par1][d, :, l * 128:(l + 1) * 128]
            for i0 in range(0, len(vun), NCH):
                grp = vun[i0:i0 + NCH]
                acc = []
                for n, (r, l) in enumerate(grp):
                    b = kbc[0, pl.ds(r * 8, 8), :] * qrow(l, 0)
                    lk = link[n] if link[n] is not None else anchor[n % T]
                    acc.append(jnp.where(never, lk, b))
                for d in range(1, DH):
                    for n, (r, l) in enumerate(grp):
                        acc[n] = acc[n] + kbc[d, pl.ds(r * 8, 8), :] * qrow(l, d)
                for n, (r, l) in enumerate(grp):
                    sout[1][pl.ds(NM + r * 8, 8), l * 128:(l + 1) * 128] = acc[n]
                    if run[n][0] == l:
                        run[n] = (l, jnp.maximum(run[n][1], acc[n]))
                    else:
                        if run[n][0] is not None:
                            vmx[run[n][0]].append(run[n][1])
                        run[n] = (l, acc[n])
                    link[n] = run[n][1]
                yield
            for n in range(NCH):
                if run[n][0] is not None:
                    vmx[run[n][0]].append(run[n][1])

        gen = vpu_gen()
        total_steps = -(-len(vun) // NCH)
        state = {"g": 0, "done": 0}

        def tick():
            state["g"] += 1
            want = (state["g"] * total_steps) // len(pv_units)
            while state["done"] < want:
                next(gen)
                state["done"] += 1

        def qk(w, r0, n):
            qm = pltpu.bitcast((was if w == 0 else wbs)[par1][...], bf16)
            if w == 0:
                kblk = pltpu.bitcast(ka[g1, pl.ds(r0 // 2, n // 2), :], bf16)
            else:
                kblk = pltpu.bitcast(kb[pl.ds(r0 // 2, n // 2), :], bf16)[:, :qm.shape[0]]
            s = jnp.dot(kblk, qm, preferred_element_type=f32)
            sout[w][pl.ds(r0, n), :] = s
            if not anchor:
                anchor.extend(s[0:8, l * 128:(l + 1) * 128] for l in range(T))
            sm = jnp.max(s.reshape(n // 8, 8, QB), axis=0)
            mx[w] = sm if w not in mx else jnp.maximum(mx[w], sm)

        def pv(w, c):
            ks = pl.ds(c * KC, KC)
            x = (sin[w][ks, :].reshape(KC // 8, 8, QB) - min_[w][...][None]).reshape(KC, QB)
            p = jnp.exp2(x)
            if w == 1:
                v = vtb[:, ks]
            else:
                rid = lax.broadcasted_iota(jnp.int32, (8, KC), 0)
                if par == 0:
                    v = jnp.concatenate([vta[hp, 0:16, ks], jnp.where(rid == 4, 1.0, vta[hp, 16:24, ks])], axis=0)
                else:
                    v = jnp.concatenate([jnp.where(rid == 0, 1.0, vta[hp, 16:24, ks]), vta[hp, 24:40, ks]], axis=0)
            d_ = jnp.dot(v, p, preferred_element_type=f32)
            accs[w] = d_ if w not in accs else accs[w] + d_
            if c == NK - 1:
                a = accs[w]
                if w == 0 and par == 1:
                    o = a * (1.0 / a[0:1, :])
                    ota[hp, DH:2 * DH, :] = o[4:24]
                else:
                    o = a * (1.0 / a[DH:DH + 1, :])
                    (ota if w == 0 else otb)[hp, par * DH:(par + 1) * DH, :] = o[0:DH]
            if do1:
                tick()

        nq_, np_ = len(qk_units), len(pv_units)
        iq = 0
        for ip in range(np_):
            while iq < nq_ and iq * np_ <= ip * nq_:
                qk(*qk_units[iq])
                iq += 1
            pv(*pv_units[ip])
        while iq < nq_:
            qk(*qk_units[iq])
            iq += 1
        if do1:
            for _ in gen:
                pass
            if NVG:
                vm = [functools.reduce(jnp.maximum, v) for v in vmx]
                mx[1] = jnp.maximum(mx[1], jnp.concatenate(vm, axis=1))
            for w in (0, 1):
                mout[w][...] = jnp.broadcast_to(jnp.max(mx[w], axis=0, keepdims=True), (8, QB))
            prep((j1 + 1) % NITEMS, par)

    buf0 = ((sa0, sb0), (ma0, mb0))
    buf1 = ((sa1, sb1), (ma1, mb1))

    def out_copy(qi):
        slot = qi % 2
        return pltpu.make_async_copy(obuf.at[slot], out_h.at[pl.ds(qi * QB, QB), :], osem.at[slot])

    def out_proj(qi):
        slot = qi % 2

        @pl.when(qi >= 2)
        def _():
            out_copy(qi - 2).wait()
        oa = ota[...].reshape(D, QB).astype(bf16)
        obuf[slot, :, 0:D] = lax.dot_general(oa, woa[...], TN, preferred_element_type=f32).astype(bf16)
        ob = otb[...].reshape(D, QB).astype(bf16)
        obuf[slot, :, D:2 * D] = lax.dot_general(ob, wob[...], TN, preferred_element_type=f32).astype(bf16)
        out_copy(qi).start()

    prep(jnp.int32(0), 0)
    item(0, 1, jnp.int32(0), None, buf0[0], None, buf0[1], do2=False)

    def body(j, carry):
        @pl.when(j % 2 == 0)
        def _():
            item(j, 0, j + 1, buf0[0], buf1[0], buf0[1], buf1[1])

        @pl.when(j % 2 == 1)
        def _():
            item(j, 1, j + 1, buf1[0], buf0[0], buf1[1], buf0[1])

        @pl.when(j % H == H - 1)
        def _():
            out_proj(j // H)
        return carry

    lax.fori_loop(0, NITEMS - 1, body, 0)
    item(jnp.int32(NITEMS - 1), 1, None, buf1[0], None, buf1[1], None, do1=False)
    out_proj(jnp.int32(NQ - 1))
    out_copy(NQ - 2).wait()
    out_copy(NQ - 1).wait()


@jax.jit
def pallas_concat_heads__softmax_full_mha__grouped_kv_mqa__prompt_kernel(
        A_x, A_wqkv, A_wo, B_x, B_wq, B_wk, B_wv, B_wo):
    V = pltpu.VMEM
    scratch = [
        V((S, D), bf16), V((D, 3 * D), bf16), V((D, D), bf16), V((S, D), bf16), V((D, D), bf16),
        V((D, DH), bf16), V((D, DH), bf16), V((D, D), bf16),
        V((2 * D, D), bf16), V((D + 128, D), bf16), V((D, 768), bf16), V((D, 128), bf16),
        V((NQ, D, QB), f32), V((NQ * T, D, 128), f32), V((6, S // 2, 128), u32), V((S // 2, 128), u32),
        V((H // 2, 2 * DH, S), f32), V((24, S), f32), V((H // 2, 2 * DH, QB), f32), V((H // 2, 2 * DH, QB), f32),
        V((DH, max(NV, 8), 128), f32),
    ] + [V((S, QB), f32)] * 4 + [V((8, QB), f32)] * 4 + [
        V((DH, 8, QB), f32), V((DH, 8, QB), f32), V((64, QB), u32), V((64, QB), u32), V((16, QB), u32), V((24, QB), u32),
        V((2, QB, 2 * D), bf16), pltpu.SMEM((3, H), jnp.int32),
        pltpu.SemaphoreType.DMA((8,)), pltpu.SemaphoreType.DMA((2,)),
    ]
    out = pl.pallas_call(
        _kernel,
        out_shape=jax.ShapeDtypeStruct((S, 2 * D), bf16),
        in_specs=[pl.BlockSpec(memory_space=pl.ANY)] * 8,
        out_specs=pl.BlockSpec(memory_space=pl.ANY),
        scratch_shapes=scratch,
        compiler_params=pltpu.CompilerParams(vmem_limit_bytes=110 * 1024 * 1024),
    )(A_x.reshape(S, D), A_wqkv, A_wo, B_x.reshape(S, D), B_wq, B_wk, B_wv, B_wo)
    return out.reshape(1, S, 2 * D)
```

```python
import functools
import math
import os

import jax
import jax.numpy as jnp
from jax import lax
import jax.experimental.pallas as pl
import jax.experimental.pallas.tpu as pltpu

S = 2048
D = 640
H = 32
DH = 20
QB = 512
T = QB // 128
NQ = S // QB
KC = 128
NK = S // KC
QSCALE = (DH ** -0.5) * math.log2(math.e)
WIN = (0, 120, 240, 360, 480, 512)
ONE = (127, 127, 127, 127, 127, 0)
NVG = int(os.environ.get("NVG", 78))
NCH = int(os.environ.get("NCH", 2))
DBL = int(os.environ.get("DBL", 7))
FORCE = int(os.environ.get("FORCE", 0))
DMAV = int(os.environ.get("DMAV", 0))
OSPLIT = int(os.environ.get("OSPLIT", 1))
KPAD = int(os.environ.get("KPAD", 3))
KOFF = int(os.environ.get("KOFF", 2))
UA = int(os.environ.get("UA", 2))
NBC = 640
NITEMS = NQ * H
INFLATE = 1.0 + 2.0 ** -6
LMIN = 2.0 ** -30
ONES2 = 0x3F803F80

f32 = jnp.float32
bf16 = jnp.bfloat16
u32 = jnp.uint32
NT = (((1,), (1,)), ((), ()))
TN = (((0,), (0,)), ((), ()))


def _colbcast(row):
    return jnp.broadcast_to(row, (128, 128)).T


def _kernel(xa_h, wqkv_h, woa_h, xb_h, wq_h, wkt_h, wvt_h, wob_h,
            out_h,
            xa, wqkv, woa, xb, wq, wkt, wvt, wob, wtb,
            qta, qtb, ka, kb, vta, vtb, ota, otb, ra, rb, kbc, kca, kcb,
            sa0, sa1, sb0, sb1, sx,
            qr0, qr1, wa0, wa1, wb0, wb1, lmin,
            obuf, tab, isem, osem):
    def cp(i, src, dst):
        return pltpu.make_async_copy(src, dst, isem.at[i])

    def cp_rows(base, src, dst, r):
        rows = pl.ds(r * QB, QB)
        return pltpu.make_async_copy(src.at[rows, :], dst.at[rows, :], isem.at[base + r])

    c_b = [cp(0, wq_h, wq), cp(1, wkt_h, wkt), cp(2, wvt_h, wvt)]
    c_a = cp(3, wqkv_h, wqkv)
    c_wo = [cp(4, woa_h, woa), cp(5, wob_h, wob)]
    for c in c_b:
        c.start()
    cp_rows(6, xb_h, xb, 0).start()

    for h in range(H):
        g = min(h // 6, 5)
        tab[0, h] = g
        tab[1, h] = WIN[g]
        tab[2, h] = h * DH - WIN[g]
        tab[3, h] = ONE[g]
        tab[4, h] = 0

    def start_rest():
        for r in range(1, NQ):
            cp_rows(6, xb_h, xb, r).start()
        c_a.start()
        for r in range(NQ):
            cp_rows(10, xa_h, xa, r).start()
        for c in c_wo:
            c.start()

    if not DMAV:
        start_rest()
    lmin[...] = jnp.full(lmin.shape, 1.0, f32)
    ra[...] = jnp.full(ra.shape, 1.0, f32)
    rb[...] = jnp.full(rb.shape, 1.0, f32)

    for c in c_b:
        c.wait()
    if DMAV:
        start_rest()
    zpad = jnp.zeros((4, D), bf16)
    wtb[0:(D + 48) // 2, :] = pltpu.bitcast(jnp.concatenate([wkt[...], zpad, wvt[...], zpad, wq[...].T], axis=0), u32)

    def proj_b(r, kabs):
        cp_rows(6, xb_h, xb, r).wait()
        xblk = xb[pl.ds(pl.multiple_of(r * QB, QB), QB), :]
        qv = lax.dot_general(pltpu.bitcast(wtb[0:(D + 48) // 2, :], bf16), xblk, NT, preferred_element_type=f32)
        k = jnp.concatenate([qv[0:24], jnp.zeros((8, QB), f32)], axis=0).T.astype(bf16)
        v = qv[24:48]
        q = qv[48:]
        kabs = jnp.maximum(kabs, jnp.max(jnp.abs(k.astype(f32)).reshape(QB // 8, 8, 32), axis=0))
        lane = lax.broadcasted_iota(jnp.int32, (QB // 2, 32), 1)
        kb[pl.ds(pl.multiple_of(r * (QB // 2), QB // 2), QB // 2), :] = jnp.where(
            lane == DH, jnp.uint32(ONES2), pltpu.bitcast(k, u32))
        rid = lax.broadcasted_iota(jnp.int32, (24, QB), 0)
        vtb[r] = jnp.where(rid == DH, 1.0, v)
        qtb[r] = (q * QSCALE).astype(bf16).astype(f32)
        return kabs

    kabs = lax.fori_loop(0, NQ, proj_b, jnp.zeros((8, 32), f32))
    kabs = jnp.max(kabs, axis=0, keepdims=True) * INFLATE
    kcb[...] = _colbcast(jnp.concatenate([kabs, jnp.zeros((1, 96), f32)], axis=1))[0:32]

    c_a.wait()

    def proj_a(r, kabs):
        xblk = xa[pl.ds(pl.multiple_of(r * QB, QB), QB), :]
        k = jnp.dot(xblk, wqkv[:, D:2 * D], preferred_element_type=f32).astype(bf16)
        kabs = jnp.maximum(kabs, jnp.max(jnp.abs(k.astype(f32)).reshape(QB // 8, 8, D), axis=0))
        ku = pltpu.bitcast(k, u32)
        lane = lax.broadcasted_iota(jnp.int32, (QB // 2, 128), 1)
        for g in range(6):
            ka[g, pl.ds(pl.multiple_of(r * (QB // 2), QB // 2), QB // 2), :] = jnp.where(
                lane == ONE[g], jnp.uint32(ONES2), ku[:, WIN[g]:WIN[g] + 128])
        nb = NBC // NQ
        kf = pltpu.bitcast(kb[pl.ds(pl.multiple_of((S - NBC) // 2 + r * (nb // 2), 8), nb // 2), :], bf16).astype(f32)
        for d in range(DH):
            kbc[d, pl.ds(pl.multiple_of(r * nb + 8 * KOFF, 8), nb), :] = jnp.broadcast_to(kf[:, d:d + 1], (nb, 128))
        wt = jnp.concatenate([wqkv[:, 0:D].T, wqkv[:, 2 * D:3 * D].T], axis=0)
        qv = lax.dot_general(wt, xblk, NT, preferred_element_type=f32)
        qta[r] = qv[:D] * QSCALE
        vta[r] = qv[D:].reshape(H // 2, 2 * DH, QB)
        return kabs

    def proj_a2(i, kabs):
        for u in range(UA):
            cp_rows(10, xa_h, xa, i * UA + u).wait()
        for u in range(UA):
            kabs = proj_a(i * UA + u, kabs)
        return kabs

    kabs = lax.fori_loop(0, NQ // UA, proj_a2, jnp.zeros((8, D), f32))
    kabs = jnp.max(kabs, axis=0, keepdims=True) * INFLATE
    for g in range(D // 128):
        kca[g * 128:(g + 1) * 128, :] = _colbcast(kabs[:, g * 128:(g + 1) * 128])

    qrs = (qr0, qr1)
    was = (wa0, wa1)
    wbs = (wb0, wb1)
    sbuf = ((sa0, sb0), (sa1, sb1))

    def prep(j2, par2, exact):
        qi = j2 >> 5
        h = j2 & (H - 1)
        hs = pl.multiple_of((h >> 1) * 2 * DH + 16 * par2, 8)
        r24 = lax.broadcasted_iota(jnp.int32, (24, QB), 0)
        st = pl.multiple_of(tab[1, h], 8)
        lo = tab[2, h]
        rows = lax.broadcasted_iota(jnp.int32, (128, QB), 0)
        w = jnp.where((rows >= lo) & (rows < lo + DH), qta[qi, pl.ds(st, 128), :], 0.0)
        if not exact:
            t = jnp.abs(qta[qi, pl.ds(hs, 24), :]) * jnp.concatenate([kca[pl.ds(hs, 24), :]] * T, axis=1)
            t = jnp.where((r24 < DH) if par2 == 0 else (r24 >= 4), t, 0.0)
            nb = -jnp.sum(t, axis=0, keepdims=True)
            r8 = lax.broadcasted_iota(jnp.int32, (8, QB), 0)
            one = tab[3, h]
            w = jnp.concatenate([jnp.where(r8 == one, nb, w[0:8]), w[8:120],
                                 jnp.where(r8 + 120 == one, nb, w[120:128])], axis=0)
        was[par2][...] = pltpu.bitcast(w.astype(bf16), u32)
        q = qtb[qi, pl.ds(hs, 24), :]
        if par2:
            q = jnp.concatenate([q[4:24], q[0:4]], axis=0)
        q = jnp.where(r24 < DH, q, 0.0)
        if not exact:
            nb = -jnp.sum(jnp.abs(q) * jnp.concatenate([kcb[0:24, :]] * T, axis=1), axis=0, keepdims=True)
            nb = nb.astype(bf16).astype(f32)
            q = jnp.where(r24 == DH, nb, q)
            for d in range(DH + 1):
                qrs[par2][d] = jnp.broadcast_to(q[d:d + 1], (8, QB))
        wbs[par2][...] = pltpu.bitcast(jnp.concatenate([q, jnp.zeros((8, QB), f32)], axis=0).astype(bf16), u32)

    def vslab(w, par, hp, blk, cols):
        if w == 1:
            return vtb[blk, :, cols]
        mid = vta[blk, hp, 16:24, cols]
        rid = lax.broadcasted_iota(jnp.int32, mid.shape, 0)
        if par == 0:
            return jnp.concatenate([vta[blk, hp, 0:16, cols], jnp.where(rid == 4, 1.0, mid)], axis=0)
        return jnp.concatenate([jnp.where(rid == 0, 1.0, mid), vta[blk, hp, 24:40, cols]], axis=0)

    def normalize(j, par):
        hp = (j & (H - 1)) >> 1
        for w in (0, 1):
            a = (ra if w == 0 else rb)[...]
            odd_a = w == 0 and par == 1
            den = a[0:1, :] if odd_a else a[DH:DH + 1, :]
            lmin[w:w + 1, :] = jnp.minimum(lmin[w:w + 1, :], den)
            o = a * (1.0 / den)
            (ota if w == 0 else otb)[hp, par * DH:(par + 1) * DH, :] = o[4:24] if odd_a else o[0:DH]

    def block(j, par, do1=True, do2=True, nvg=NVG):
        nm = S - nvg * 8
        par1 = 1 - par
        g1 = tab[0, (j + 1) & (H - 1)]
        hp = (j & (H - 1)) >> 1
        never = lax.broadcasted_iota(jnp.int32, (8, 128), 0) > (tab[4, 0] + 1000)
        link = [None] * NCH
        sout = sbuf[par1]
        accs = {}
        vun = [(r, l) for l in range(T) for r in range(nvg)] if do1 else []
        rounds = [vun[i:i + NCH] for i in range(0, len(vun), NCH)]
        ns = DH - DBL
        dbl = set((i * ns) // DBL + 1 for i in range(DBL)) if DBL else set()
        steps = []
        for i in range(ns):
            d0 = sum(len(s) for s in steps)
            steps.append(list(range(d0, d0 + (2 if i in dbl else 1))))

        def vpu_gen():
            for grp in rounds:
                acc = []
                for c, (r, l) in enumerate(grp):
                    b = qrs[par1][DH, :, l * 128:(l + 1) * 128]
                    acc.append(b if link[c] is None else jnp.where(never, link[c], b))
                for st in steps:
                    for c, (r, l) in enumerate(grp):
                        ts = [kbc[d, pl.ds(NBC - nvg * 8 + r * 8 + 8 * KOFF, 8), :] * qrs[par1][d, :, l * 128:(l + 1) * 128]
                              for d in st]
                        acc[c] = acc[c] + functools.reduce(jnp.add, ts)
                for c, (r, l) in enumerate(grp):
                    sout[1][pl.ds(nm + r * 8, 8), l * 128:(l + 1) * 128] = acc[c]
                    link[c] = acc[c]
                yield

        def qk(w, r0, nr):
            qm = pltpu.bitcast((was if w == 0 else wbs)[par1][...], bf16)
            kblk = ka[g1, pl.ds(r0 // 2, nr // 2), :] if w == 0 else kb[pl.ds(r0 // 2, nr // 2), :]
            sout[w][pl.ds(r0, nr), :] = jnp.dot(pltpu.bitcast(kblk, bf16), qm, preferred_element_type=f32)

        def pv(w, c):
            p = jnp.exp2(sbuf[par][w][pl.ds(c * KC, KC), :])
            v = vslab(w, par, hp, c // T, slice((c % T) * KC, (c % T + 1) * KC))
            d_ = jnp.dot(v, p, preferred_element_type=f32)
            accs[w] = d_ if c == 0 else accs[w] + d_
            if c == NK - 1 and w == 0:
                ra[...] = accs[w]

        qus = []
        pus = []
        for c in range(NK):
            if do1:
                b0 = ((c * (nm // 16)) // NK) * 16
                b1 = (((c + 1) * (nm // 16)) // NK) * 16
                qus += [(1, b0, b1 - b0), (0, c * KC, KC)]
            if do2:
                pus += [(0, c), (1, c)]
        if not do2:
            qus = qus[0::2] + qus[1::2]
        gen = vpu_gen()
        if do1:
            prep((j + 2) & (NITEMS - 1), par, False)
        if do2:
            normalize(j - 1, par1)
        done = 0
        for i in range(2 * NK):
            if do1:
                qk(*qus[i])
            if do2:
                pv(*pus[i])
            while done < ((i + 1) * len(rounds)) // (2 * NK):
                next(gen)
                done += 1
        if do2:
            a = accs[1]
            top = a[0:8]
            if vun:
                tl = functools.reduce(jnp.maximum, link)
                top = jnp.concatenate([jnp.where(never, tl, top[:, 0:128]), top[:, 128:]], axis=1)
            rb[...] = jnp.concatenate([top, a[8:]], axis=0)

    def exact_item(j, par):
        prep(j, par, True)
        h = j & (H - 1)
        for w in (0, 1):
            qm = pltpu.bitcast((was if w == 0 else wbs)[par][...], bf16)

            def scores(b, m, w=w, qm=qm):
                rows = pl.ds(pl.multiple_of(b * (QB // 2), QB // 2), QB // 2)
                kblk = ka[tab[0, h], rows, :] if w == 0 else kb[rows, :]
                sc = jnp.dot(pltpu.bitcast(kblk, bf16), qm, preferred_element_type=f32)
                sx[pl.ds(pl.multiple_of(b * QB, QB), QB), :] = sc
                return jnp.maximum(m, jnp.max(sc.reshape(QB // 8, 8, QB), axis=0))

            m = lax.fori_loop(0, NQ, scores, jnp.full((8, QB), -jnp.inf, f32))
            m = jnp.max(m, axis=0, keepdims=True)

            def weighted(b, acc, w=w, m=m):
                p = jnp.exp2(sx[pl.ds(pl.multiple_of(b * QB, QB), QB), :] - m)
                return acc + jnp.dot(vslab(w, par, h >> 1, b, slice(None)), p, preferred_element_type=f32)

            (ra if w == 0 else rb)[...] = lax.fori_loop(0, NQ, weighted, jnp.zeros((24, QB), f32))
        normalize(j, par)

    def out_copy(qi, w):
        slot = qi & 1
        return pltpu.make_async_copy(obuf.at[2 * slot + w], out_h.at[pl.ds(qi * QB, QB), w * D:(w + 1) * D],
                                     osem.at[2 * slot + w])

    def out_proj(qi):
        slot = qi & 1

        @pl.when(qi >= 2)
        def _():
            out_copy(qi - 2, 0).wait()
            out_copy(qi - 2, 1).wait()
        normalize(jnp.int32(H - 1), 1)
        oa = ota[...].reshape(D, QB).astype(bf16)
        obuf[2 * slot] = lax.dot_general(oa, woa[...], TN, preferred_element_type=f32).astype(bf16)
        if OSPLIT:
            out_copy(qi, 0).start()
        ob = otb[...].reshape(D, QB).astype(bf16)
        obuf[2 * slot + 1] = lax.dot_general(ob, wob[...], TN, preferred_element_type=f32).astype(bf16)
        if not OSPLIT:
            out_copy(qi, 0).start()
        out_copy(qi, 1).start()

    prep(jnp.int32(0), 0, False)
    block(jnp.int32(-1), 1, do2=False, nvg=0)

    def one_pass(p, carry):
        @pl.when(tab[4, 1] == 0)
        def _():
            def body(i, c2):
                j = 2 * i

                @pl.when(p == 0)
                def _():
                    block(j, 0)

                @pl.when((p == 0) & (j + 1 < NITEMS - 1))
                def _():
                    block(j + 1, 1)

                @pl.when((p != 0) | ((j & (H - 1)) == H - 2))
                def _():
                    @pl.when((p == 0) & (j + 1 == NITEMS - 1))
                    def _():
                        block(j + 1, 1, do1=False)

                    @pl.when(p != 0)
                    def _():
                        exact_item(j, 0)
                        exact_item(j + 1, 1)

                    @pl.when((j & (H - 1)) == H - 2)
                    def _():
                        out_proj(j >> 5)
                return c2

            lax.fori_loop(0, NITEMS // 2, body, 0)
            ok = jnp.min(jnp.where(lmin[...] >= LMIN, 1.0, 0.0)) > (0.5 if not FORCE else 2.0)
            tab[4, 1] = jnp.where(ok, 1, 0)
            for qi in (NQ - 2, NQ - 1):
                for w in (0, 1):
                    out_copy(qi, w).wait()
        return carry

    for c in c_wo:
        c.wait()
    lax.fori_loop(0, 2, one_pass, 0)


@jax.jit
def pallas_concat_heads__softmax_full_mha__grouped_kv_mqa__prompt_kernel(
        A_x, A_wqkv, A_wo, B_x, B_wq, B_wk, B_wv, B_wo):
    V = pltpu.VMEM
    scratch = [
        V((S, D), bf16), V((D, 3 * D), bf16), V((D, D), bf16), V((S, D), bf16), V((D, D), bf16),
        V((DH, D), bf16), V((DH, D), bf16), V((D, D), bf16), V(((D + 64) // 2, D), u32),
        V((NQ, D, QB), f32), V((NQ, D, QB), f32), V((6, S // 2, 128), u32), V((S // 2, 32), u32),
        V((NQ, H // 2, 2 * DH, QB), f32), V((NQ, 24, QB), f32),
        V((H // 2, 2 * DH, QB), f32), V((H // 2, 2 * DH, QB), f32), V((24, QB), f32), V((24, QB), f32),
        V((DH, NBC + 8 * KPAD, 128), f32), V((D, 128), f32), V((32, 128), f32),
    ] + [V((S, QB), f32)] * 5 + [
        V((DH + 1, 8, QB), f32), V((DH + 1, 8, QB), f32),
        V((64, QB), u32), V((64, QB), u32), V((16, QB), u32), V((16, QB), u32), V((8, QB), f32),
        V((4, QB, D), bf16), pltpu.SMEM((5, H), jnp.int32),
        pltpu.SemaphoreType.DMA((14,)), pltpu.SemaphoreType.DMA((4,)),
    ]
    out = pl.pallas_call(
        _kernel,
        out_shape=jax.ShapeDtypeStruct((S, 2 * D), bf16),
        in_specs=[pl.BlockSpec(memory_space=pl.ANY)] * 8,
        out_specs=pl.BlockSpec(memory_space=pl.ANY),
        scratch_shapes=scratch,
        compiler_params=pltpu.CompilerParams(vmem_limit_bytes=110 * 1024 * 1024),
    )(A_x.reshape(S, D), A_wqkv, A_wo, B_x.reshape(S, D), B_wq, B_wk.T, B_wv.T, B_wo)
    return out.reshape(1, S, 2 * D)
```

```python
import functools
import math

import jax
import jax.numpy as jnp
from jax import lax
import jax.experimental.pallas as pl
import jax.experimental.pallas.tpu as pltpu

S = 2048
D = 640
H = 32
DH = 20
QB = 512
T = QB // 128
NQ = S // QB
KC = 128
NK = S // KC
NITEMS = NQ * H
QSCALE = (DH ** -0.5) * math.log2(math.e)
KW = 48
NVG = 78
PNVG = 64
NCH = 2
DBL = 7
DOFF = 2
NBC = 640
KPAD = 3
KOFF = 2
UA = 2
MIDLAG = 8
INFLATE = 1.0 + 2.0 ** -6
LMIN = 2.0 ** -30
ONES2 = 0x3F803F80

f32 = jnp.float32
bf16 = jnp.bfloat16
u32 = jnp.uint32
NT = (((1,), (1,)), ((), ()))
TN = (((0,), (0,)), ((), ()))


def _colbcast(row):
    return jnp.broadcast_to(row, (128, 128)).T


def _kernel(xa_h, wqkv_h, woa_h, xb_h, wq_h, wkt_h, wvt_h, wob_h,
            out_h,
            xa, wqkv, woa, xb, wq, wkt, wvt, wob, wtb,
            qta, qtb, ka, kb, vta, vtb, ota, otb, ra, rb, kbc, kca, kcb,
            s0, s1, s2, s3, s4, s5, s6, s7, sx,
            qr0, qr1, qr2, qr3, wa0, wa1, wa2, wa3, wb0, wb1, wb2, wb3, ra1, rb1, okv,
            part, obuf, tab, isem, osem):
    def cp(i, src, dst):
        return pltpu.make_async_copy(src, dst, isem.at[i])

    def cp_rows(base, src, dst, r):
        rows = pl.ds(r * QB, QB)
        return pltpu.make_async_copy(src.at[rows, :], dst.at[rows, :], isem.at[base + r])

    c_b = [cp(0, wq_h, wq), cp(1, wkt_h, wkt), cp(2, wvt_h, wvt)]
    c_a = cp(3, wqkv_h, wqkv)
    c_wo = [cp(4, woa_h, woa), cp(5, wob_h, wob)]
    for c in c_b:
        c.start()
    cp_rows(6, xb_h, xb, 0).start()

    tab[0] = 0
    tab[1] = 0

    for r in range(1, NQ):
        cp_rows(6, xb_h, xb, r).start()
    c_a.start()
    for r in range(NQ):
        cp_rows(10, xa_h, xa, r).start()
    for c in c_wo:
        c.start()
    okv[...] = jnp.full(okv.shape, 1.0, f32)
    ra[...] = jnp.full(ra.shape, 1.0, f32)
    rb[...] = jnp.full(rb.shape, 1.0, f32)
    ra1[...] = jnp.full(ra.shape, 1.0, f32)
    rb1[...] = jnp.full(rb.shape, 1.0, f32)

    for c in c_b:
        c.wait()
    zpad = jnp.zeros((4, D), bf16)
    wtb[0:(D + 48) // 2, :] = pltpu.bitcast(
        jnp.concatenate([wkt[...], zpad, wvt[...], zpad, wq[...].T], axis=0), u32)

    def proj_b(r, kabs):
        cp_rows(6, xb_h, xb, r).wait()
        xblk = xb[pl.ds(pl.multiple_of(r * QB, QB), QB), :]
        qv = lax.dot_general(pltpu.bitcast(wtb[0:(D + 48) // 2, :], bf16), xblk, NT,
                             preferred_element_type=f32)
        k = jnp.concatenate([qv[0:24], jnp.zeros((8, QB), f32)], axis=0).T.astype(bf16)
        v = qv[24:48]
        q = qv[48:]
        kabs = jnp.maximum(kabs, jnp.max(jnp.abs(k.astype(f32)).reshape(QB // 8, 8, 32), axis=0))
        lane = lax.broadcasted_iota(jnp.int32, (QB // 2, 32), 1)
        kb[pl.ds(pl.multiple_of(r * (QB // 2), QB // 2), QB // 2), :] = jnp.where(
            lane == DH, jnp.uint32(ONES2), pltpu.bitcast(k, u32))
        rid = lax.broadcasted_iota(jnp.int32, (24, QB), 0)
        vtb[r, 0] = jnp.where(rid == DH, 1.0, v)
        vtb[r, 1] = jnp.where(rid == 0, 1.0, qv[20:44])
        qtb[r] = (q * QSCALE).astype(bf16).astype(f32)
        return kabs

    kabs = lax.fori_loop(0, NQ, proj_b, jnp.zeros((8, 32), f32))
    kabs = jnp.max(kabs, axis=0, keepdims=True) * INFLATE
    kcb[...] = _colbcast(jnp.concatenate([kabs, jnp.zeros((1, 96), f32)], axis=1))[0:32]

    c_a.wait()

    def proj_a(r, kabs):
        xblk = xa[pl.ds(pl.multiple_of(r * QB, QB), QB), :]
        k = jnp.dot(xblk, wqkv[:, D:2 * D], preferred_element_type=f32).astype(bf16)
        kabs = jnp.maximum(kabs, jnp.max(jnp.abs(k.astype(f32)).reshape(QB // 8, 8, D), axis=0))
        ku = pltpu.bitcast(k, u32)
        ku = jnp.concatenate([ku, ku[:, 0:128]], axis=1)
        lane = lax.broadcasted_iota(jnp.int32, (QB // 2, KW), 1)
        for g in range(H // 2):
            ka[g, pl.ds(pl.multiple_of(r * (QB // 2), QB // 2), QB // 2), :] = jnp.where(
                lane == 2 * DH, jnp.uint32(ONES2), ku[:, 2 * DH * g:2 * DH * g + KW])
        nb = NBC // NQ
        kf = pltpu.bitcast(kb[pl.ds(pl.multiple_of((S - NBC) // 2 + r * (nb // 2), 8), nb // 2), :],
                           bf16).astype(f32)
        for d in range(DH):
            kbc[d, pl.ds(pl.multiple_of(r * nb + 8 * KOFF, 8), nb), :] = jnp.broadcast_to(kf[:, d:d + 1], (nb, 128))
        wt = jnp.concatenate([wqkv[:, 0:D].T, wqkv[:, 2 * D:3 * D].T], axis=0)
        qv = lax.dot_general(wt, xblk, NT, preferred_element_type=f32)
        qta[r] = qv[:D] * QSCALE
        vta[r] = qv[D:].reshape(H // 2, 2 * DH, QB)
        return kabs

    def proj_a2(i, kabs):
        for u in range(UA):
            cp_rows(10, xa_h, xa, i * UA + u).wait()
        for u in range(UA):
            kabs = proj_a(i * UA + u, kabs)
        return kabs

    kabs = lax.fori_loop(0, NQ // UA, proj_a2, jnp.zeros((8, D), f32))
    kabs = jnp.max(kabs, axis=0, keepdims=True) * INFLATE
    for g in range(D // 128):
        kca[g * 128:(g + 1) * 128, :] = _colbcast(kabs[:, g * 128:(g + 1) * 128])

    qrs = (qr0, qr1, qr2, qr3)
    was = (wa0, wa1, wa2, wa3)
    wbs = (wb0, wb1, wb2, wb3)
    sbuf = ((s0, s1), (s2, s3), (s4, s5), (s6, s7))
    raw = ((ra, rb), (ra1, rb1))

    def prep(j2, slot, exact):
        par2 = slot & 1
        qi = j2 >> 5
        h = j2 & (H - 1)
        hs = pl.multiple_of((h >> 1) * 2 * DH + 16 * par2, 8)
        r24 = lax.broadcasted_iota(jnp.int32, (24, QB), 0)
        z8 = jnp.zeros((8, QB), f32)
        t = jnp.where((r24 < DH) if par2 == 0 else (r24 >= 4), qta[qi, pl.ds(hs, 24), :], 0.0)
        last = z8
        if not exact:
            nb = -jnp.sum(jnp.abs(t) * jnp.concatenate([kca[pl.ds(hs, 24), :]] * T, axis=1), axis=0, keepdims=True)
            last = jnp.where(lax.broadcasted_iota(jnp.int32, (8, QB), 0) == 0, nb, 0.0)
        w = jnp.concatenate([t, z8, z8, last] if par2 == 0 else [z8, z8, t, last], axis=0)
        was[slot][0:24, :] = pltpu.bitcast(w.astype(bf16), u32)
        q = qtb[qi, pl.ds(hs, 24), :]
        if par2:
            q = jnp.concatenate([q[4:24], q[0:4]], axis=0)
        q = jnp.where(r24 < DH, q, 0.0)
        if not exact:
            nb = -jnp.sum(jnp.abs(q) * jnp.concatenate([kcb[0:24, :]] * T, axis=1), axis=0, keepdims=True)
            nb = nb.astype(bf16).astype(f32)
            q = jnp.where(r24 == DH, nb, q)
            for d in range(DH + 1):
                qrs[slot][d] = jnp.broadcast_to(q[d:d + 1], (8, QB))
        wbs[slot][...] = pltpu.bitcast(jnp.concatenate([q, jnp.zeros((8, QB), f32)], axis=0).astype(bf16), u32)

    def wload(w, s):
        return pltpu.bitcast(wbs[s][...] if w else was[s][0:24, :], bf16)

    def vslab(w, par, hp, blk, cols):
        if w == 1:
            return vtb[blk, par, :, cols]
        mid = vta[blk, hp, 16:24, cols]
        rid = lax.broadcasted_iota(jnp.int32, mid.shape, 0)
        if par == 0:
            return jnp.concatenate([vta[blk, hp, 0:16, cols], jnp.where(rid == 4, 1.0, mid)], axis=0)
        return jnp.concatenate([jnp.where(rid == 0, 1.0, mid), vta[blk, hp, 24:40, cols]], axis=0)

    def normalize(j, par, ws=(0, 1)):
        hp = (j & (H - 1)) >> 1
        for w in ws:
            a = raw[par][w][...]
            den = a[0:1, :] if par else a[DH:DH + 1, :]
            okv[w:w + 1, :] = jnp.where(den >= LMIN, okv[w:w + 1, :], -1.0)
            o = a * (1.0 / den)
            (ota if w == 0 else otb)[hp, par * DH:(par + 1) * DH, :] = o[4:24] if par else o[0:DH]

    def block(j, s0_, do1=True, do2=True, nvg=NVG, extra=(), mid=None):
        nm = S - nvg * 8
        hp = (j & (H - 1)) >> 1
        never = lax.broadcasted_iota(jnp.int32, (8, 128), 0) > (tab[0] + 1000)
        link = [None] * NCH
        accs = {}
        vun = [(u, r, l) for u in range(2) for l in range(T) for r in range(nvg)] if do1 else []
        rounds = [vun[i:i + NCH] for i in range(0, len(vun), NCH)]
        ns = DH - DBL
        dbl = set(((i * ns) // DBL + DOFF) % ns for i in range(DBL))
        steps = []
        for i in range(ns):
            d0 = sum(len(s) for s in steps)
            steps.append(list(range(d0, d0 + (2 if i in dbl else 1))))
        s1_ = (s0_ + 2) & 3
        g1 = ((j + 2) & (H - 1)) >> 1

        def vpu_gen():
            for grp in rounds:
                acc = []
                for c, (u, r, l) in enumerate(grp):
                    b = qrs[s1_ + u][DH, :, l * 128:(l + 1) * 128]
                    acc.append(b if link[c] is None else jnp.where(never, link[c], b))
                for st in steps:
                    for c, (u, r, l) in enumerate(grp):
                        ts = [kbc[d, pl.ds(NBC - nvg * 8 + r * 8 + 8 * KOFF, 8), :]
                              * qrs[s1_ + u][d, :, l * 128:(l + 1) * 128] for d in st]
                        acc[c] = acc[c] + functools.reduce(jnp.add, ts)
                for c, (u, r, l) in enumerate(grp):
                    sbuf[s1_ + u][1][pl.ds(nm + r * 8, 8), l * 128:(l + 1) * 128] = acc[c]
                    link[c] = acc[c]
                yield

        def tie(x):
            tl = functools.reduce(jnp.maximum, link)
            return jnp.concatenate([jnp.where(never, tl, x[:, 0:128]), x[:, 128:]], axis=1)

        def qk(u, w, r0, nr):
            qm = wload(w, s1_ + u)
            kblk = ka[g1, pl.ds(r0 // 2, nr // 2), :] if w == 0 else kb[pl.ds(r0 // 2, nr // 2), :]
            sc = jnp.dot(pltpu.bitcast(kblk, bf16), qm, preferred_element_type=f32)
            if not do2 and (u, w, r0, nr) == qus[-1]:
                for _ in gen:
                    pass
                sc = jnp.concatenate([sc[:nr - 8], tie(sc[nr - 8:])], axis=0)
            sbuf[s1_ + u][w][pl.ds(r0, nr), :] = sc

        def pv(u, w, c):
            p = jnp.exp2(sbuf[s0_ + u][w][pl.ds(c * KC, KC), :])
            v = vslab(w, u, hp, c // T, slice((c % T) * KC, (c % T + 1) * KC))
            d_ = jnp.dot(v, p, preferred_element_type=f32)
            accs[w] = d_ if c == 0 else accs[w] + d_
            if c == NK - 1 and not (w == 1 and u == 1):
                raw[u][w][...] = accs[w]

        qus = []
        pus = []
        for u in range(2):
            for c in range(NK):
                b0 = ((c * (nm // 16)) // NK) * 16
                b1 = (((c + 1) * (nm // 16)) // NK) * 16
                qus += [(u, 1, b0, b1 - b0), (u, 0, c * KC, KC)]
                pus += [(u, 0, c), (u, 1, c)]
        if not do2:
            qus = qus[0::2] + qus[1::2]
        if mid is not None:
            pus = pus[0::2] + pus[1::2]
        gen = vpu_gen()
        for u in range(2):
            if do1:
                prep((j + 4 + u) & (NITEMS - 1), s0_ + u, False)
            if do2:
                normalize(j - 2 + u, u)
        done = 0
        for i in range(4 * NK):
            if mid is not None and i == 2 * NK + MIDLAG:
                mid()
            if do1:
                qk(*qus[i])
            for e in extra[(i * len(extra)) // (4 * NK):((i + 1) * len(extra)) // (4 * NK)]:
                e()
            if do2:
                pv(*pus[i])
            while done < ((i + 1) * len(rounds)) // (4 * NK) and (do2 or i < 4 * NK - 1):
                next(gen)
                done += 1
        if do2:
            a = accs[1]
            raw[1][1][...] = jnp.concatenate([tie(a[0:8]), a[8:]], axis=0) if do1 else a

    def exact_item(j, par):
        prep(j, par, True)
        h = j & (H - 1)
        for w in (0, 1):
            qm = wload(w, par)

            def scores(b, m, w=w, qm=qm):
                rows = pl.ds(pl.multiple_of(b * (QB // 2), QB // 2), QB // 2)
                kblk = ka[h >> 1, rows, :] if w == 0 else kb[rows, :]
                sc = jnp.dot(pltpu.bitcast(kblk, bf16), qm, preferred_element_type=f32)
                sx[pl.ds(pl.multiple_of(b * QB, QB), QB), :] = sc
                return jnp.maximum(m, jnp.max(sc.reshape(QB // 8, 8, QB), axis=0))

            m = lax.fori_loop(0, NQ, scores, jnp.full((8, QB), -jnp.inf, f32))
            m = jnp.max(m, axis=0, keepdims=True)

            def weighted(b, acc, w=w, m=m):
                p = jnp.exp2(sx[pl.ds(pl.multiple_of(b * QB, QB), QB), :] - m)
                return acc + jnp.dot(vslab(w, par, h >> 1, b, slice(None)), p, preferred_element_type=f32)

            raw[par][w][...] = lax.fori_loop(0, NQ, weighted, jnp.zeros((24, QB), f32))
        normalize(j, par)

    def out_copy(qi, w):
        slot = qi & 1
        return pltpu.make_async_copy(obuf.at[2 * slot + w], out_h.at[pl.ds(qi * QB, QB), w * D:(w + 1) * D],
                                     osem.at[2 * slot + w])

    def out_proj(qi):
        slot = qi & 1

        @pl.when(qi >= 2)
        def _():
            out_copy(qi - 2, 0).wait()
            out_copy(qi - 2, 1).wait()
        normalize(jnp.int32(H - 2), 0)
        normalize(jnp.int32(H - 1), 1)
        oa = ota[...].reshape(D, QB).astype(bf16)
        obuf[2 * slot] = lax.dot_general(oa, woa[...], TN, preferred_element_type=f32).astype(bf16)
        out_copy(qi, 0).start()
        ob = otb[...].reshape(D, QB).astype(bf16)
        obuf[2 * slot + 1] = lax.dot_general(ob, wob[...], TN, preferred_element_type=f32).astype(bf16)
        out_copy(qi, 1).start()

    def final_block():
        qi = NQ - 1
        kp = 512
        out_copy(qi - 2, 0).wait()
        out_copy(qi - 2, 1).wait()
        lhs = {}

        def unit(w, m, n):
            if (w, m) not in lhs:
                o = (ota if w == 0 else otb)[0:13, :, m * 128:(m + 1) * 128].reshape(13 * 2 * DH, 128)[0:kp]
                lhs[w, m] = o.T.astype(bf16)
            part[w, m * 128:(m + 1) * 128, n * 128:(n + 1) * 128] = jnp.dot(
                lhs[w, m], (woa if w == 0 else wob)[0:kp, n * 128:(n + 1) * 128], preferred_element_type=f32)

        extra = [functools.partial(unit, w, m, n) for w in (0, 1) for m in range(T) for n in range(D // 128)]

        def finish(w):
            normalize(jnp.int32(H - 2), 0, (w,))
            normalize(jnp.int32(H - 1), 1, (w,))
            o = (ota if w == 0 else otb)[12:16].reshape(4 * 2 * DH, QB)[kp - 12 * 2 * DH:].astype(bf16)
            rest = lax.dot_general(o, (woa if w == 0 else wob)[kp:, :], TN, preferred_element_type=f32)
            obuf[2 * (qi & 1) + w] = (part[w] + rest).astype(bf16)
            out_copy(qi, w).start()

        block(jnp.int32(NITEMS - 2), 2, do1=False, extra=extra, mid=functools.partial(finish, 0))
        finish(1)

    prep(jnp.int32(0), 0, False)
    prep(jnp.int32(1), 1, False)
    block(jnp.int32(-2), 2, do2=False, nvg=PNVG)

    def one_pass(p, carry):
        @pl.when(tab[1] == 0)
        def _():
            def body(i, c2):
                j = 4 * i

                @pl.when(p == 0)
                def _():
                    block(j, 0)

                @pl.when((p == 0) & (j + 2 < NITEMS - 2))
                def _():
                    block(j + 2, 2)

                @pl.when((p != 0) | ((j & (H - 1)) == H - 4))
                def _():
                    @pl.when((p == 0) & (j + 2 == NITEMS - 2))
                    def _():
                        final_block()

                    @pl.when(p != 0)
                    def _():
                        def pair(u, c3):
                            exact_item(j + 2 * u, 0)
                            exact_item(j + 2 * u + 1, 1)
                            return c3
                        lax.fori_loop(0, 2, pair, 0)

                    @pl.when(((j & (H - 1)) == H - 4) & ((p != 0) | (j + 2 != NITEMS - 2)))
                    def _():
                        out_proj(j >> 5)
                return c2

            lax.fori_loop(0, NITEMS // 4, body, 0)
            tab[1] = jnp.where(jnp.min(okv[...]) > 0.5, 1, 0)
            for qi in (NQ - 2, NQ - 1):
                for w in (0, 1):
                    out_copy(qi, w).wait()
        return carry

    for c in c_wo:
        c.wait()
    lax.fori_loop(0, 2, one_pass, 0)


@jax.jit
def pallas_concat_heads__softmax_full_mha__grouped_kv_mqa__prompt_kernel(
        A_x, A_wqkv, A_wo, B_x, B_wq, B_wk, B_wv, B_wo):
    V = pltpu.VMEM
    scratch = [
        V((S, D), bf16), V((D, 3 * D), bf16), V((D, D), bf16), V((S, D), bf16), V((D, D), bf16),
        V((DH, D), bf16), V((DH, D), bf16), V((D, D), bf16), V(((D + 64) // 2, D), u32),
        V((NQ, D, QB), f32), V((NQ, D, QB), f32), V((H // 2, S // 2, KW), u32), V((S // 2, 32), u32),
        V((NQ, H // 2, 2 * DH, QB), f32), V((NQ, 2, 24, QB), f32),
        V((H // 2, 2 * DH, QB), f32), V((H // 2, 2 * DH, QB), f32), V((24, QB), f32), V((24, QB), f32),
        V((DH, NBC + 8 * KPAD, 128), f32), V((D, 128), f32), V((32, 128), f32),
    ] + [V((S, QB), f32)] * 9 + [V((DH + 1, 8, QB), f32)] * 4 + [V((32, QB), u32)] * 4 + [
        V((16, QB), u32)] * 4 + [V((24, QB), f32)] * 2 + [
        V((8, QB), f32),
        V((2, QB, D), f32), V((4, QB, D), bf16), pltpu.SMEM((2,), jnp.int32),
        pltpu.SemaphoreType.DMA((14,)), pltpu.SemaphoreType.DMA((4,)),
    ]
    out = pl.pallas_call(
        _kernel,
        out_shape=jax.ShapeDtypeStruct((S, 2 * D), bf16),
        in_specs=[pl.BlockSpec(memory_space=pl.ANY)] * 8,
        out_specs=pl.BlockSpec(memory_space=pl.ANY),
        scratch_shapes=scratch,
        compiler_params=pltpu.CompilerParams(vmem_limit_bytes=110 * 1024 * 1024),
    )(A_x.reshape(S, D), A_wqkv, A_wo, B_x.reshape(S, D), B_wq, B_wk.T, B_wv.T, B_wo)
    return out.reshape(1, S, 2 * D)
```

```python
import functools
import math

import jax
import jax.numpy as jnp
from jax import lax
import jax.experimental.pallas as pl
import jax.experimental.pallas.tpu as pltpu

S = 2048
D = 640
H = 32
DH = 20
QB = 512
T = QB // 128
NQ = S // QB
KC = 128
NK = S // KC
NITEMS = NQ * H
QSCALE = (DH ** -0.5) * math.log2(math.e)
KW = 48
NVG = 78
PNVG = 64
NCH = 2
DBL = 7
DOFF = 1
NBC = 640
KPAD = 3
KOFF = 2
UA = 2
MIDLAG = 8
INFLATE = 1.0 + 2.0 ** -6
LMIN = 2.0 ** -30
ONES2 = 0x3F803F80

f32 = jnp.float32
bf16 = jnp.bfloat16
u32 = jnp.uint32
NT = (((1,), (1,)), ((), ()))
TN = (((0,), (0,)), ((), ()))


def _colbcast(row):
    return jnp.broadcast_to(row, (128, 128)).T


def _kernel(xa_h, wqkv_h, woa_h, xb_h, wq_h, wkt_h, wvt_h, wob_h,
            out_h,
            xa, wqkv, woa, xb, wq, wkt, wvt, wob, wtb,
            qta, qtb, ka, kb, vta, vtb, ota, otb, ra, rb, kbc, kca, kcb,
            s0, s1, s2, s3, s4, s5, s6, s7, sx,
            qr0, qr1, qr2, qr3, wa0, wa1, wa2, wa3, wb0, wb1, wb2, wb3, ra1, rb1, okv,
            part, obuf, tab, isem, osem):
    def cp(i, src, dst):
        return pltpu.make_async_copy(src, dst, isem.at[i])

    def cp_rows(base, src, dst, r):
        rows = pl.ds(r * QB, QB)
        return pltpu.make_async_copy(src.at[rows, :], dst.at[rows, :], isem.at[base + r])

    c_b = [cp(0, wq_h, wq), cp(1, wkt_h, wkt), cp(2, wvt_h, wvt)]
    c_a = cp(3, wqkv_h, wqkv)
    c_wo = [cp(4, woa_h, woa), cp(5, wob_h, wob)]
    for c in c_b:
        c.start()
    cp_rows(6, xb_h, xb, 0).start()

    tab[0] = 0
    tab[1] = 0

    for r in range(1, NQ):
        cp_rows(6, xb_h, xb, r).start()
    c_a.start()
    for r in range(NQ):
        cp_rows(10, xa_h, xa, r).start()
    for c in c_wo:
        c.start()
    okv[...] = jnp.full(okv.shape, 1.0, f32)
    ra[...] = jnp.full(ra.shape, 1.0, f32)
    rb[...] = jnp.full(rb.shape, 1.0, f32)
    ra1[...] = jnp.full(ra.shape, 1.0, f32)
    rb1[...] = jnp.full(rb.shape, 1.0, f32)

    for c in c_b:
        c.wait()
    zpad = jnp.zeros((4, D), bf16)
    wtb[0:(D + 48) // 2, :] = pltpu.bitcast(
        jnp.concatenate([wkt[...], zpad, wvt[...], zpad, wq[...].T], axis=0), u32)

    def proj_b(r, kabs):
        cp_rows(6, xb_h, xb, r).wait()
        xblk = xb[pl.ds(pl.multiple_of(r * QB, QB), QB), :]
        qv = lax.dot_general(pltpu.bitcast(wtb[0:(D + 48) // 2, :], bf16), xblk, NT,
                             preferred_element_type=f32)
        k = jnp.concatenate([qv[0:24], jnp.zeros((8, QB), f32)], axis=0).T.astype(bf16)
        v = qv[24:48]
        q = qv[48:]
        kabs = jnp.maximum(kabs, jnp.max(jnp.abs(k.astype(f32)).reshape(QB // 8, 8, 32), axis=0))
        lane = lax.broadcasted_iota(jnp.int32, (QB // 2, 32), 1)
        kb[pl.ds(pl.multiple_of(r * (QB // 2), QB // 2), QB // 2), :] = jnp.where(
            lane == DH, jnp.uint32(ONES2), pltpu.bitcast(k, u32))
        rid = lax.broadcasted_iota(jnp.int32, (24, QB), 0)
        vtb[r, 0] = jnp.where(rid == DH, 1.0, v)
        vtb[r, 1] = jnp.where(rid == 0, 1.0, qv[20:44])
        qtb[r] = (q * QSCALE).astype(bf16).astype(f32)
        return kabs

    kabs = lax.fori_loop(0, NQ, proj_b, jnp.zeros((8, 32), f32))
    kabs = jnp.max(kabs, axis=0, keepdims=True) * INFLATE
    kcb[...] = _colbcast(jnp.concatenate([kabs, jnp.zeros((1, 96), f32)], axis=1))[0:32]

    c_a.wait()

    def proj_a(r, kabs):
        xblk = xa[pl.ds(pl.multiple_of(r * QB, QB), QB), :]
        k = jnp.dot(xblk, wqkv[:, D:2 * D], preferred_element_type=f32).astype(bf16)
        kabs = jnp.maximum(kabs, jnp.max(jnp.abs(k.astype(f32)).reshape(QB // 8, 8, D), axis=0))
        ku = pltpu.bitcast(k, u32)
        ku = jnp.concatenate([ku, ku[:, 0:128]], axis=1)
        lane = lax.broadcasted_iota(jnp.int32, (QB // 2, KW), 1)
        for g in range(H // 2):
            ka[g, pl.ds(pl.multiple_of(r * (QB // 2), QB // 2), QB // 2), :] = jnp.where(
                lane == 2 * DH, jnp.uint32(ONES2), ku[:, 2 * DH * g:2 * DH * g + KW])
        nb = NBC // NQ
        kf = pltpu.bitcast(kb[pl.ds(pl.multiple_of((S - NBC) // 2 + r * (nb // 2), 8), nb // 2), :],
                           bf16).astype(f32)
        for d in range(DH):
            kbc[d, pl.ds(pl.multiple_of(r * nb + 8 * KOFF, 8), nb), :] = jnp.broadcast_to(kf[:, d:d + 1], (nb, 128))
        wt = jnp.concatenate([wqkv[:, 0:D].T, wqkv[:, 2 * D:3 * D].T], axis=0)
        qv = lax.dot_general(wt, xblk, NT, preferred_element_type=f32)
        qta[r] = qv[:D] * QSCALE
        vta[r] = qv[D:].reshape(H // 2, 2 * DH, QB)
        return kabs

    def proj_a2(i, kabs):
        for u in range(UA):
            cp_rows(10, xa_h, xa, i * UA + u).wait()
        for u in range(UA):
            kabs = proj_a(i * UA + u, kabs)
        return kabs

    kabs = lax.fori_loop(0, NQ // UA, proj_a2, jnp.zeros((8, D), f32))
    kabs = jnp.max(kabs, axis=0, keepdims=True) * INFLATE
    for g in range(D // 128):
        kca[g * 128:(g + 1) * 128, :] = _colbcast(kabs[:, g * 128:(g + 1) * 128])

    qrs = (qr0, qr1, qr2, qr3)
    was = (wa0, wa1, wa2, wa3)
    wbs = (wb0, wb1, wb2, wb3)
    sbuf = ((s0, s1), (s2, s3), (s4, s5), (s6, s7))
    raw = ((ra, rb), (ra1, rb1))

    def prep(j2, slot, exact):
        par2 = slot & 1
        qi = j2 >> 5
        h = j2 & (H - 1)
        hs = pl.multiple_of((h >> 1) * 2 * DH + 16 * par2, 8)
        r24 = lax.broadcasted_iota(jnp.int32, (24, QB), 0)
        z8 = jnp.zeros((8, QB), f32)
        t = jnp.where((r24 < DH) if par2 == 0 else (r24 >= 4), qta[qi, pl.ds(hs, 24), :], 0.0)
        last = z8
        if not exact:
            nb = -jnp.sum(jnp.abs(t) * jnp.concatenate([kca[pl.ds(hs, 24), :]] * T, axis=1), axis=0, keepdims=True)
            last = jnp.where(lax.broadcasted_iota(jnp.int32, (8, QB), 0) == 0, nb, 0.0)
        w = jnp.concatenate([t, z8, z8, last] if par2 == 0 else [z8, z8, t, last], axis=0)
        was[slot][0:24, :] = pltpu.bitcast(w.astype(bf16), u32)
        q = qtb[qi, pl.ds(hs, 24), :]
        if par2:
            q = jnp.concatenate([q[4:24], q[0:4]], axis=0)
        q = jnp.where(r24 < DH, q, 0.0)
        if not exact:
            nb = -jnp.sum(jnp.abs(q) * jnp.concatenate([kcb[0:24, :]] * T, axis=1), axis=0, keepdims=True)
            nb = nb.astype(bf16).astype(f32)
            q = jnp.where(r24 == DH, nb, q)
            for d in range(DH + 1):
                qrs[slot][d] = jnp.broadcast_to(q[d:d + 1], (8, QB))
        wbs[slot][...] = pltpu.bitcast(jnp.concatenate([q, jnp.zeros((8, QB), f32)], axis=0).astype(bf16), u32)

    def wload(w, s):
        return pltpu.bitcast(wbs[s][...] if w else was[s][0:24, :], bf16)

    def vslab(w, par, hp, blk, cols):
        if w == 1:
            return vtb[blk, par, :, cols]
        mid = vta[blk, hp, 16:24, cols]
        rid = lax.broadcasted_iota(jnp.int32, mid.shape, 0)
        if par == 0:
            return jnp.concatenate([vta[blk, hp, 0:16, cols], jnp.where(rid == 4, 1.0, mid)], axis=0)
        return jnp.concatenate([jnp.where(rid == 0, 1.0, mid), vta[blk, hp, 24:40, cols]], axis=0)

    def normalize(j, par, ws=(0, 1)):
        hp = (j & (H - 1)) >> 1
        for w in ws:
            a = raw[par][w][...]
            den = a[0:1, :] if par else a[DH:DH + 1, :]
            okv[w:w + 1, :] = jnp.where(den >= LMIN, okv[w:w + 1, :], -1.0)
            o = a * (1.0 / den)
            (ota if w == 0 else otb)[hp, par * DH:(par + 1) * DH, :] = o[4:24] if par else o[0:DH]

    def block(j, s0_, do1=True, do2=True, nvg=NVG, extra=(), mid=None):
        nm = S - nvg * 8
        hp = (j & (H - 1)) >> 1
        never = lax.broadcasted_iota(jnp.int32, (8, 128), 0) > (tab[0] + 1000)
        link = []
        accs = {}
        rounds = [(u, r, l) for u in range(2) for l in range(T) for r in range(0, nvg, NCH)] if do1 else []
        ns = DH - DBL
        dbl = set(((i * ns) // DBL + DOFF) % ns for i in range(DBL))
        steps = []
        for i in range(ns):
            d0 = sum(len(s) for s in steps)
            steps.append(list(range(d0, d0 + (2 if i in dbl else 1))))
        s1_ = (s0_ + 2) & 3
        g1 = ((j + 2) & (H - 1)) >> 1

        def vpu_gen():
            for u, r, l in rounds:
                cols = slice(l * 128, (l + 1) * 128)
                qq = qrs[s1_ + u][:, :, cols]
                kk = kbc[:, pl.ds(NBC - nvg * 8 + r * 8 + 8 * KOFF, 8 * NCH), :]
                kk = kk.reshape(DH, NCH, 8, 128)
                acc = jnp.broadcast_to(qq[DH][None], (NCH, 8, 128))
                if link:
                    acc = jnp.where(never[None], link.pop(), acc)
                for st in steps:
                    acc = acc + functools.reduce(jnp.add, [kk[d] * qq[d][None] for d in st])
                sbuf[s1_ + u][1][pl.ds(nm + r * 8, 8 * NCH), cols] = acc.reshape(8 * NCH, 128)
                link.append(acc)
                yield

        def tie(x):
            return jnp.concatenate([jnp.where(never, jnp.max(link[0], axis=0), x[:, 0:128]), x[:, 128:]], axis=1)

        def qk(u, w, r0, nr):
            qm = wload(w, s1_ + u)
            kblk = ka[g1, pl.ds(r0 // 2, nr // 2), :] if w == 0 else kb[pl.ds(r0 // 2, nr // 2), :]
            sc = jnp.dot(pltpu.bitcast(kblk, bf16), qm, preferred_element_type=f32)
            if not do2 and (u, w, r0, nr) == qus[-1]:
                for _ in gen:
                    pass
                sc = jnp.concatenate([sc[:nr - 8], tie(sc[nr - 8:])], axis=0)
            sbuf[s1_ + u][w][pl.ds(r0, nr), :] = sc

        def pv(u, w, c):
            p = jnp.exp2(sbuf[s0_ + u][w][pl.ds(c * KC, KC), :])
            v = vslab(w, u, hp, c // T, slice((c % T) * KC, (c % T + 1) * KC))
            d_ = jnp.dot(v, p, preferred_element_type=f32)
            accs[w] = d_ if c == 0 else accs[w] + d_
            if c == NK - 1 and not (w == 1 and u == 1):
                raw[u][w][...] = accs[w]

        qus = []
        pus = []
        for u in range(2):
            for c in range(NK):
                b0 = ((c * (nm // 16)) // NK) * 16
                b1 = (((c + 1) * (nm // 16)) // NK) * 16
                qus += [(u, 1, b0, b1 - b0), (u, 0, c * KC, KC)]
                pus += [(u, 0, c), (u, 1, c)]
        if not do2:
            qus = qus[0::2] + qus[1::2]
        if mid is not None:
            pus = pus[0::2] + pus[1::2]
        gen = vpu_gen()
        for u in range(2):
            if do1:
                prep((j + 4 + u) & (NITEMS - 1), s0_ + u, False)
            if do2:
                normalize(j - 2 + u, u)
        done = 0
        for i in range(4 * NK):
            if mid is not None and i == 2 * NK + MIDLAG:
                mid()
            if do1:
                qk(*qus[i])
            for e in extra[(i * len(extra)) // (4 * NK):((i + 1) * len(extra)) // (4 * NK)]:
                e()
            if do2:
                pv(*pus[i])
            while done < ((i + 1) * len(rounds)) // (4 * NK) and (do2 or i < 4 * NK - 1):
                next(gen)
                done += 1
        if do2:
            a = accs[1]
            raw[1][1][...] = jnp.concatenate([tie(a[0:8]), a[8:]], axis=0) if do1 else a

    def exact_item(j, par):
        prep(j, par, True)
        h = j & (H - 1)
        for w in (0, 1):
            qm = wload(w, par)

            def scores(b, m, w=w, qm=qm):
                rows = pl.ds(pl.multiple_of(b * (QB // 2), QB // 2), QB // 2)
                kblk = ka[h >> 1, rows, :] if w == 0 else kb[rows, :]
                sc = jnp.dot(pltpu.bitcast(kblk, bf16), qm, preferred_element_type=f32)
                sx[pl.ds(pl.multiple_of(b * QB, QB), QB), :] = sc
                return jnp.maximum(m, jnp.max(sc.reshape(QB // 8, 8, QB), axis=0))

            m = lax.fori_loop(0, NQ, scores, jnp.full((8, QB), -jnp.inf, f32))
            m = jnp.max(m, axis=0, keepdims=True)

            def weighted(b, acc, w=w, m=m):
                p = jnp.exp2(sx[pl.ds(pl.multiple_of(b * QB, QB), QB), :] - m)
                return acc + jnp.dot(vslab(w, par, h >> 1, b, slice(None)), p, preferred_element_type=f32)

            raw[par][w][...] = lax.fori_loop(0, NQ, weighted, jnp.zeros((24, QB), f32))
        normalize(j, par)

    def out_copy(qi, w):
        slot = qi & 1
        return pltpu.make_async_copy(obuf.at[2 * slot + w], out_h.at[pl.ds(qi * QB, QB), w * D:(w + 1) * D],
                                     osem.at[2 * slot + w])

    def out_proj(qi):
        slot = qi & 1

        @pl.when(qi >= 2)
        def _():
            out_copy(qi - 2, 0).wait()
            out_copy(qi - 2, 1).wait()
        normalize(jnp.int32(H - 2), 0)
        normalize(jnp.int32(H - 1), 1)
        oa = ota[...].reshape(D, QB).astype(bf16)
        obuf[2 * slot] = lax.dot_general(oa, woa[...], TN, preferred_element_type=f32).astype(bf16)
        out_copy(qi, 0).start()
        ob = otb[...].reshape(D, QB).astype(bf16)
        obuf[2 * slot + 1] = lax.dot_general(ob, wob[...], TN, preferred_element_type=f32).astype(bf16)
        out_copy(qi, 1).start()

    def final_block():
        qi = NQ - 1
        kp = 512
        out_copy(qi - 2, 0).wait()
        out_copy(qi - 2, 1).wait()
        lhs = {}

        def unit(w, m, n):
            if (w, m) not in lhs:
                o = (ota if w == 0 else otb)[0:13, :, m * 128:(m + 1) * 128].reshape(13 * 2 * DH, 128)[0:kp]
                lhs[w, m] = o.T.astype(bf16)
            part[w, m * 128:(m + 1) * 128, n * 128:(n + 1) * 128] = jnp.dot(
                lhs[w, m], (woa if w == 0 else wob)[0:kp, n * 128:(n + 1) * 128], preferred_element_type=f32)

        extra = [functools.partial(unit, w, m, n) for w in (0, 1) for m in range(T) for n in range(D // 128)]

        def finish(w):
            normalize(jnp.int32(H - 2), 0, (w,))
            normalize(jnp.int32(H - 1), 1, (w,))
            o = (ota if w == 0 else otb)[12:16].reshape(4 * 2 * DH, QB)[kp - 12 * 2 * DH:].astype(bf16)
            rest = lax.dot_general(o, (woa if w == 0 else wob)[kp:, :], TN, preferred_element_type=f32)
            obuf[2 * (qi & 1) + w] = (part[w] + rest).astype(bf16)
            out_copy(qi, w).start()

        block(jnp.int32(NITEMS - 2), 2, do1=False, extra=extra, mid=functools.partial(finish, 0))
        finish(1)

    prep(jnp.int32(0), 0, False)
    prep(jnp.int32(1), 1, False)
    block(jnp.int32(-2), 2, do2=False, nvg=PNVG)

    def one_pass(p, carry):
        @pl.when(tab[1] == 0)
        def _():
            def body(i, c2):
                j = 4 * i

                @pl.when(p == 0)
                def _():
                    block(j, 0)

                @pl.when((p == 0) & (j + 2 < NITEMS - 2))
                def _():
                    block(j + 2, 2)

                @pl.when((p != 0) | ((j & (H - 1)) == H - 4))
                def _():
                    @pl.when((p == 0) & (j + 2 == NITEMS - 2))
                    def _():
                        final_block()

                    @pl.when(p != 0)
                    def _():
                        def pair(u, c3):
                            exact_item(j + 2 * u, 0)
                            exact_item(j + 2 * u + 1, 1)
                            return c3
                        lax.fori_loop(0, 2, pair, 0)

                    @pl.when(((j & (H - 1)) == H - 4) & ((p != 0) | (j + 2 != NITEMS - 2)))
                    def _():
                        out_proj(j >> 5)
                return c2

            lax.fori_loop(0, NITEMS // 4, body, 0)
            tab[1] = jnp.where(jnp.min(okv[...]) > 0.5, 1, 0)
            for qi in (NQ - 2, NQ - 1):
                for w in (0, 1):
                    out_copy(qi, w).wait()
        return carry

    for c in c_wo:
        c.wait()
    lax.fori_loop(0, 2, one_pass, 0)


@jax.jit
def pallas_concat_heads__softmax_full_mha__grouped_kv_mqa__prompt_kernel(
        A_x, A_wqkv, A_wo, B_x, B_wq, B_wk, B_wv, B_wo):
    V = pltpu.VMEM
    scratch = [
        V((S, D), bf16), V((D, 3 * D), bf16), V((D, D), bf16), V((S, D), bf16), V((D, D), bf16),
        V((DH, D), bf16), V((DH, D), bf16), V((D, D), bf16), V(((D + 64) // 2, D), u32),
        V((NQ, D, QB), f32), V((NQ, D, QB), f32), V((H // 2, S // 2, KW), u32), V((S // 2, 32), u32),
        V((NQ, H // 2, 2 * DH, QB), f32), V((NQ, 2, 24, QB), f32),
        V((H // 2, 2 * DH, QB), f32), V((H // 2, 2 * DH, QB), f32), V((24, QB), f32), V((24, QB), f32),
        V((DH, NBC + 8 * KPAD, 128), f32), V((D, 128), f32), V((32, 128), f32),
    ] + [V((S, QB), f32)] * 9 + [V((DH + 1, 8, QB), f32)] * 4 + [V((32, QB), u32)] * 4 + [
        V((16, QB), u32)] * 4 + [V((24, QB), f32)] * 2 + [
        V((8, QB), f32),
        V((2, QB, D), f32), V((4, QB, D), bf16), pltpu.SMEM((2,), jnp.int32),
        pltpu.SemaphoreType.DMA((14,)), pltpu.SemaphoreType.DMA((4,)),
    ]
    out = pl.pallas_call(
        _kernel,
        out_shape=jax.ShapeDtypeStruct((S, 2 * D), bf16),
        in_specs=[pl.BlockSpec(memory_space=pl.ANY)] * 8,
        out_specs=pl.BlockSpec(memory_space=pl.ANY),
        scratch_shapes=scratch,
        compiler_params=pltpu.CompilerParams(vmem_limit_bytes=110 * 1024 * 1024),
    )(A_x.reshape(S, D), A_wqkv, A_wo, B_x.reshape(S, D), B_wq, B_wk.T, B_wv.T, B_wo)
    return out.reshape(1, S, 2 * D)
```

```python
import functools
import math

import jax
import jax.numpy as jnp
from jax import lax
import jax.experimental.pallas as pl
import jax.experimental.pallas.tpu as pltpu

S = 2048
D = 640
H = 32
DH = 20
QB = 512
T = QB // 128
NQ = S // QB
KC = 128
NK = S // KC
NITEMS = NQ * H
QSCALE = (DH ** -0.5) * math.log2(math.e)
KW = 48
NVG = 78
PNVG = 64
NCH = 2
DBL = 7
DOFF = 0
BACK = 3
NBC = 640
KPAD = 3
KOFF = 2
UA = 2
MIDLAG = 8
INFLATE = 1.0 + 2.0 ** -6
LMIN = 2.0 ** -30
ONES2 = 0x3F803F80

f32 = jnp.float32
bf16 = jnp.bfloat16
u32 = jnp.uint32
NT = (((1,), (1,)), ((), ()))
TN = (((0,), (0,)), ((), ()))


def _colbcast(row):
    return jnp.broadcast_to(row, (128, 128)).T


def _kernel(xa_h, wqkv_h, woa_h, xb_h, wq_h, wkt_h, wvt_h, wob_h,
            out_h,
            xa, wqkv, woa, xb, wq, wkt, wvt, wob, wtb,
            qta, qtb, ka, kb, vta, vtb, ota, otb, ra, rb, kbc, kca, kcb,
            s0, s1, s2, s3, s4, s5, s6, s7, sx,
            qr0, qr1, qr2, qr3, wa0, wa1, wa2, wa3, wb0, wb1, wb2, wb3, ra1, rb1, okv,
            part, obuf, tab, isem, osem):
    def cp(i, src, dst):
        return pltpu.make_async_copy(src, dst, isem.at[i])

    def cp_rows(base, src, dst, r):
        rows = pl.ds(r * QB, QB)
        return pltpu.make_async_copy(src.at[rows, :], dst.at[rows, :], isem.at[base + r])

    c_b = [cp(0, wq_h, wq), cp(1, wkt_h, wkt), cp(2, wvt_h, wvt)]
    c_a = cp(3, wqkv_h, wqkv)
    c_wo = [cp(4, woa_h, woa), cp(5, wob_h, wob)]
    for c in c_b:
        c.start()
    cp_rows(6, xb_h, xb, 0).start()

    tab[0] = 0
    tab[1] = 0

    for r in range(1, NQ):
        cp_rows(6, xb_h, xb, r).start()
    c_a.start()
    for r in range(NQ):
        cp_rows(10, xa_h, xa, r).start()
    for c in c_wo:
        c.start()
    okv[...] = jnp.full(okv.shape, 1.0, f32)
    ra[...] = jnp.full(ra.shape, 1.0, f32)
    rb[...] = jnp.full(rb.shape, 1.0, f32)
    ra1[...] = jnp.full(ra.shape, 1.0, f32)
    rb1[...] = jnp.full(rb.shape, 1.0, f32)

    for c in c_b:
        c.wait()
    zpad = jnp.zeros((4, D), bf16)
    wtb[0:(D + 48) // 2, :] = pltpu.bitcast(
        jnp.concatenate([wkt[...], zpad, wvt[...], zpad, wq[...].T], axis=0), u32)

    def proj_b(r, kabs):
        cp_rows(6, xb_h, xb, r).wait()
        xblk = xb[pl.ds(pl.multiple_of(r * QB, QB), QB), :]
        qv = lax.dot_general(pltpu.bitcast(wtb[0:(D + 48) // 2, :], bf16), xblk, NT,
                             preferred_element_type=f32)
        k = jnp.concatenate([qv[0:24], jnp.zeros((8, QB), f32)], axis=0).T.astype(bf16)
        v = qv[24:48]
        q = qv[48:]
        kabs = jnp.maximum(kabs, jnp.max(jnp.abs(k.astype(f32)).reshape(QB // 8, 8, 32), axis=0))
        lane = lax.broadcasted_iota(jnp.int32, (QB // 2, 32), 1)
        kb[pl.ds(pl.multiple_of(r * (QB // 2), QB // 2), QB // 2), :] = jnp.where(
            lane == DH, jnp.uint32(ONES2), pltpu.bitcast(k, u32))
        rid = lax.broadcasted_iota(jnp.int32, (24, QB), 0)
        vtb[r, 0] = jnp.where(rid == DH, 1.0, v)
        vtb[r, 1] = jnp.where(rid == 0, 1.0, qv[20:44])
        qtb[r] = (q * QSCALE).astype(bf16).astype(f32)
        return kabs

    kabs = lax.fori_loop(0, NQ, proj_b, jnp.zeros((8, 32), f32))
    kabs = jnp.max(kabs, axis=0, keepdims=True) * INFLATE
    kcb[...] = _colbcast(jnp.concatenate([kabs, jnp.zeros((1, 96), f32)], axis=1))[0:32]

    c_a.wait()

    def proj_a(r, kabs):
        xblk = xa[pl.ds(pl.multiple_of(r * QB, QB), QB), :]
        k = jnp.dot(xblk, wqkv[:, D:2 * D], preferred_element_type=f32).astype(bf16)
        kabs = jnp.maximum(kabs, jnp.max(jnp.abs(k.astype(f32)).reshape(QB // 8, 8, D), axis=0))
        ku = pltpu.bitcast(k, u32)
        ku = jnp.concatenate([ku, ku[:, 0:128]], axis=1)
        lane = lax.broadcasted_iota(jnp.int32, (QB // 2, KW), 1)
        for g in range(H // 2):
            ka[g, pl.ds(pl.multiple_of(r * (QB // 2), QB // 2), QB // 2), :] = jnp.where(
                lane == 2 * DH, jnp.uint32(ONES2), ku[:, 2 * DH * g:2 * DH * g + KW])
        nb = NBC // NQ
        kf = pltpu.bitcast(kb[pl.ds(pl.multiple_of((S - NBC) // 2 + r * (nb // 2), 8), nb // 2), :],
                           bf16).astype(f32)
        for d in range(DH):
            kbc[d, pl.ds(pl.multiple_of(r * nb + 8 * KOFF, 8), nb), :] = jnp.broadcast_to(kf[:, d:d + 1], (nb, 128))
        wt = jnp.concatenate([wqkv[:, 0:D].T, wqkv[:, 2 * D:3 * D].T], axis=0)
        qv = lax.dot_general(wt, xblk, NT, preferred_element_type=f32)
        qta[r] = qv[:D] * QSCALE
        vta[r] = qv[D:].reshape(H // 2, 2 * DH, QB)
        return kabs

    def proj_a2(i, kabs):
        for u in range(UA):
            cp_rows(10, xa_h, xa, i * UA + u).wait()
        for u in range(UA):
            kabs = proj_a(i * UA + u, kabs)
        return kabs

    kabs = lax.fori_loop(0, NQ // UA, proj_a2, jnp.zeros((8, D), f32))
    kabs = jnp.max(kabs, axis=0, keepdims=True) * INFLATE
    for g in range(D // 128):
        kca[g * 128:(g + 1) * 128, :] = _colbcast(kabs[:, g * 128:(g + 1) * 128])

    qrs = (qr0, qr1, qr2, qr3)
    was = (wa0, wa1, wa2, wa3)
    wbs = (wb0, wb1, wb2, wb3)
    sbuf = ((s0, s1), (s2, s3), (s4, s5), (s6, s7))
    raw = ((ra, rb), (ra1, rb1))

    def prep(j2, slot, exact):
        par2 = slot & 1
        qi = j2 >> 5
        h = j2 & (H - 1)
        hs = pl.multiple_of((h >> 1) * 2 * DH + 16 * par2, 8)
        r24 = lax.broadcasted_iota(jnp.int32, (24, QB), 0)
        z8 = jnp.zeros((8, QB), f32)
        t = jnp.where((r24 < DH) if par2 == 0 else (r24 >= 4), qta[qi, pl.ds(hs, 24), :], 0.0)
        last = z8
        if not exact:
            nb = -jnp.sum(jnp.abs(t) * jnp.concatenate([kca[pl.ds(hs, 24), :]] * T, axis=1), axis=0, keepdims=True)
            last = jnp.where(lax.broadcasted_iota(jnp.int32, (8, QB), 0) == 0, nb, 0.0)
        w = jnp.concatenate([t, z8, z8, last] if par2 == 0 else [z8, z8, t, last], axis=0)
        was[slot][0:24, :] = pltpu.bitcast(w.astype(bf16), u32)
        q = qtb[qi, pl.ds(hs, 24), :]
        if par2:
            q = jnp.concatenate([q[4:24], q[0:4]], axis=0)
        q = jnp.where(r24 < DH, q, 0.0)
        if not exact:
            nb = -jnp.sum(jnp.abs(q) * jnp.concatenate([kcb[0:24, :]] * T, axis=1), axis=0, keepdims=True)
            nb = nb.astype(bf16).astype(f32)
            q = jnp.where(r24 == DH, nb, q)
            qrs[slot][...] = q
        wbs[slot][...] = pltpu.bitcast(jnp.concatenate([q, jnp.zeros((8, QB), f32)], axis=0).astype(bf16), u32)

    def wload(w, s):
        return pltpu.bitcast(wbs[s][...] if w else was[s][0:24, :], bf16)

    def vslab(w, par, hp, blk, cols):
        if w == 1:
            return vtb[blk, par, :, cols]
        mid = vta[blk, hp, 16:24, cols]
        rid = lax.broadcasted_iota(jnp.int32, mid.shape, 0)
        if par == 0:
            return jnp.concatenate([vta[blk, hp, 0:16, cols], jnp.where(rid == 4, 1.0, mid)], axis=0)
        return jnp.concatenate([jnp.where(rid == 0, 1.0, mid), vta[blk, hp, 24:40, cols]], axis=0)

    def normalize(j, par, ws=(0, 1)):
        hp = (j & (H - 1)) >> 1
        for w in ws:
            a = raw[par][w][...]
            den = a[0:1, :] if par else a[DH:DH + 1, :]
            okv[w:w + 1, :] = jnp.where(den >= LMIN, okv[w:w + 1, :], -1.0)
            o = a * (1.0 / den)
            (ota if w == 0 else otb)[hp, par * DH:(par + 1) * DH, :] = o[4:24] if par else o[0:DH]

    def block(j, s0_, do1=True, do2=True, nvg=NVG, extra=(), mid=None):
        nm = S - nvg * 8
        hp = (j & (H - 1)) >> 1
        never = lax.broadcasted_iota(jnp.int32, (8, 128), 0) > (tab[0] + 1000)
        hist = []
        accs = {}
        rounds = [(u, r, l) for u in range(2) for l in range(T) for r in range(0, nvg, NCH)] if do1 else []
        ns = DH - DBL
        dbl = set(((i * ns) // DBL + DOFF) % ns for i in range(DBL))
        steps = []
        for i in range(ns):
            d0 = sum(len(s) for s in steps)
            steps.append(list(range(d0, d0 + (2 if i in dbl else 1))))
        s1_ = (s0_ + 2) & 3
        g1 = ((j + 2) & (H - 1)) >> 1

        def vpu_gen():
            for u, r, l in rounds:
                cols = slice(l * 128, (l + 1) * 128)
                if r == 0:
                    q24 = jnp.where(never[None], hist[-BACK][0][None] if hist else 3.0,
                                    qrs[s1_ + u][:, cols].reshape(3, 8, 128)).reshape(24, 128)
                    qq = [jnp.broadcast_to(q24[d:d + 1], (8, 128)) for d in range(DH + 1)]
                kk = kbc[:, pl.ds(NBC - nvg * 8 + r * 8 + 8 * KOFF, 8 * NCH), :]
                kk = kk.reshape(DH, NCH, 8, 128)
                acc = jnp.broadcast_to(qq[DH][None], (NCH, 8, 128))
                if hist:
                    acc = jnp.where(never[None], hist[-1], acc)
                for st in steps:
                    acc = acc + functools.reduce(jnp.add, [kk[d] * qq[d][None] for d in st])
                sbuf[s1_ + u][1][pl.ds(nm + r * 8, 8 * NCH), cols] = acc.reshape(8 * NCH, 128)
                hist.append(acc)
                yield

        def tie(x):
            return jnp.concatenate([jnp.where(never, jnp.max(hist[-1], axis=0), x[:, 0:128]), x[:, 128:]], axis=1)

        def qk(u, w, r0, nr):
            qm = wload(w, s1_ + u)
            kblk = ka[g1, pl.ds(r0 // 2, nr // 2), :] if w == 0 else kb[pl.ds(r0 // 2, nr // 2), :]
            sc = jnp.dot(pltpu.bitcast(kblk, bf16), qm, preferred_element_type=f32)
            if not do2 and (u, w, r0, nr) == qus[-1]:
                for _ in gen:
                    pass
                sc = jnp.concatenate([sc[:nr - 8], tie(sc[nr - 8:])], axis=0)
            sbuf[s1_ + u][w][pl.ds(r0, nr), :] = sc

        def pv(u, w, c):
            p = jnp.exp2(sbuf[s0_ + u][w][pl.ds(c * KC, KC), :])
            v = vslab(w, u, hp, c // T, slice((c % T) * KC, (c % T + 1) * KC))
            d_ = jnp.dot(v, p, preferred_element_type=f32)
            accs[w] = d_ if c == 0 else accs[w] + d_
            if c == NK - 1 and not (w == 1 and u == 1):
                raw[u][w][...] = accs[w]

        qus = []
        pus = []
        for u in range(2):
            for c in range(NK):
                b0 = ((c * (nm // 16)) // NK) * 16
                b1 = (((c + 1) * (nm // 16)) // NK) * 16
                qus += [(u, 1, b0, b1 - b0), (u, 0, c * KC, KC)]
                pus += [(u, 0, c), (u, 1, c)]
        if not do2:
            qus = qus[0::2] + qus[1::2]
        if mid is not None:
            pus = pus[0::2] + pus[1::2]
        gen = vpu_gen()
        for u in range(2):
            if do1:
                prep((j + 4 + u) & (NITEMS - 1), s0_ + u, False)
            if do2:
                normalize(j - 2 + u, u)
        done = 0
        for i in range(4 * NK):
            if mid is not None and i == 2 * NK + MIDLAG:
                mid()
            if do1:
                qk(*qus[i])
            for e in extra[(i * len(extra)) // (4 * NK):((i + 1) * len(extra)) // (4 * NK)]:
                e()
            if do2:
                pv(*pus[i])
            while done < ((i + 1) * len(rounds)) // (4 * NK) and (do2 or i < 4 * NK - 1):
                next(gen)
                done += 1
        if do2:
            a = accs[1]
            raw[1][1][...] = jnp.concatenate([tie(a[0:8]), a[8:]], axis=0) if do1 else a

    def exact_item(j, par):
        prep(j, par, True)
        h = j & (H - 1)
        for w in (0, 1):
            qm = wload(w, par)

            def scores(b, m, w=w, qm=qm):
                rows = pl.ds(pl.multiple_of(b * (QB // 2), QB // 2), QB // 2)
                kblk = ka[h >> 1, rows, :] if w == 0 else kb[rows, :]
                sc = jnp.dot(pltpu.bitcast(kblk, bf16), qm, preferred_element_type=f32)
                sx[pl.ds(pl.multiple_of(b * QB, QB), QB), :] = sc
                return jnp.maximum(m, jnp.max(sc.reshape(QB // 8, 8, QB), axis=0))

            m = lax.fori_loop(0, NQ, scores, jnp.full((8, QB), -jnp.inf, f32))
            m = jnp.max(m, axis=0, keepdims=True)

            def weighted(b, acc, w=w, m=m):
                p = jnp.exp2(sx[pl.ds(pl.multiple_of(b * QB, QB), QB), :] - m)
                return acc + jnp.dot(vslab(w, par, h >> 1, b, slice(None)), p, preferred_element_type=f32)

            raw[par][w][...] = lax.fori_loop(0, NQ, weighted, jnp.zeros((24, QB), f32))
        normalize(j, par)

    def out_copy(qi, w):
        slot = qi & 1
        return pltpu.make_async_copy(obuf.at[2 * slot + w], out_h.at[pl.ds(qi * QB, QB), w * D:(w + 1) * D],
                                     osem.at[2 * slot + w])

    def out_proj(qi):
        slot = qi & 1

        @pl.when(qi >= 2)
        def _():
            out_copy(qi - 2, 0).wait()
            out_copy(qi - 2, 1).wait()
        normalize(jnp.int32(H - 2), 0)
        normalize(jnp.int32(H - 1), 1)
        oa = ota[...].reshape(D, QB).astype(bf16)
        obuf[2 * slot] = lax.dot_general(oa, woa[...], TN, preferred_element_type=f32).astype(bf16)
        out_copy(qi, 0).start()
        ob = otb[...].reshape(D, QB).astype(bf16)
        obuf[2 * slot + 1] = lax.dot_general(ob, wob[...], TN, preferred_element_type=f32).astype(bf16)
        out_copy(qi, 1).start()

    def final_block():
        qi = NQ - 1
        kp = 512
        out_copy(qi - 2, 0).wait()
        out_copy(qi - 2, 1).wait()
        lhs = {}

        def unit(w, m, n):
            if (w, m) not in lhs:
                o = (ota if w == 0 else otb)[0:13, :, m * 128:(m + 1) * 128].reshape(13 * 2 * DH, 128)[0:kp]
                lhs[w, m] = o.T.astype(bf16)
            part[w, m * 128:(m + 1) * 128, n * 128:(n + 1) * 128] = jnp.dot(
                lhs[w, m], (woa if w == 0 else wob)[0:kp, n * 128:(n + 1) * 128], preferred_element_type=f32)

        extra = [functools.partial(unit, w, m, n) for w in (0, 1) for m in range(T) for n in range(D // 128)]

        def finish(w):
            normalize(jnp.int32(H - 2), 0, (w,))
            normalize(jnp.int32(H - 1), 1, (w,))
            o = (ota if w == 0 else otb)[12:16].reshape(4 * 2 * DH, QB)[kp - 12 * 2 * DH:].astype(bf16)
            rest = lax.dot_general(o, (woa if w == 0 else wob)[kp:, :], TN, preferred_element_type=f32)
            obuf[2 * (qi & 1) + w] = (part[w] + rest).astype(bf16)
            out_copy(qi, w).start()

        block(jnp.int32(NITEMS - 2), 2, do1=False, extra=extra, mid=functools.partial(finish, 0))
        finish(1)

    prep(jnp.int32(0), 0, False)
    prep(jnp.int32(1), 1, False)
    block(jnp.int32(-2), 2, do2=False, nvg=PNVG)

    def one_pass(p, carry):
        @pl.when(tab[1] == 0)
        def _():
            def body(i, c2):
                j = 4 * i

                @pl.when(p == 0)
                def _():
                    block(j, 0)

                @pl.when((p == 0) & (j + 2 < NITEMS - 2))
                def _():
                    block(j + 2, 2)

                @pl.when((p != 0) | ((j & (H - 1)) == H - 4))
                def _():
                    @pl.when((p == 0) & (j + 2 == NITEMS - 2))
                    def _():
                        final_block()

                    @pl.when(p != 0)
                    def _():
                        def pair(u, c3):
                            exact_item(j + 2 * u, 0)
                            exact_item(j + 2 * u + 1, 1)
                            return c3
                        lax.fori_loop(0, 2, pair, 0)

                    @pl.when(((j & (H - 1)) == H - 4) & ((p != 0) | (j + 2 != NITEMS - 2)))
                    def _():
                        out_proj(j >> 5)
                return c2

            lax.fori_loop(0, NITEMS // 4, body, 0)
            tab[1] = jnp.where(jnp.min(okv[...]) > 0.5, 1, 0)
            for qi in (NQ - 2, NQ - 1):
                for w in (0, 1):
                    out_copy(qi, w).wait()
        return carry

    for c in c_wo:
        c.wait()
    lax.fori_loop(0, 2, one_pass, 0)


@jax.jit
def pallas_concat_heads__softmax_full_mha__grouped_kv_mqa__prompt_kernel(
        A_x, A_wqkv, A_wo, B_x, B_wq, B_wk, B_wv, B_wo):
    V = pltpu.VMEM
    scratch = [
        V((S, D), bf16), V((D, 3 * D), bf16), V((D, D), bf16), V((S, D), bf16), V((D, D), bf16),
        V((DH, D), bf16), V((DH, D), bf16), V((D, D), bf16), V(((D + 64) // 2, D), u32),
        V((NQ, D, QB), f32), V((NQ, D, QB), f32), V((H // 2, S // 2, KW), u32), V((S // 2, 32), u32),
        V((NQ, H // 2, 2 * DH, QB), f32), V((NQ, 2, 24, QB), f32),
        V((H // 2, 2 * DH, QB), f32), V((H // 2, 2 * DH, QB), f32), V((24, QB), f32), V((24, QB), f32),
        V((DH, NBC + 8 * KPAD, 128), f32), V((D, 128), f32), V((32, 128), f32),
    ] + [V((S, QB), f32)] * 9 + [V((24, QB), f32)] * 4 + [V((32, QB), u32)] * 4 + [
        V((16, QB), u32)] * 4 + [V((24, QB), f32)] * 2 + [
        V((8, QB), f32),
        V((2, QB, D), f32), V((4, QB, D), bf16), pltpu.SMEM((2,), jnp.int32),
        pltpu.SemaphoreType.DMA((14,)), pltpu.SemaphoreType.DMA((4,)),
    ]
    out = pl.pallas_call(
        _kernel,
        out_shape=jax.ShapeDtypeStruct((S, 2 * D), bf16),
        in_specs=[pl.BlockSpec(memory_space=pl.ANY)] * 8,
        out_specs=pl.BlockSpec(memory_space=pl.ANY),
        scratch_shapes=scratch,
        compiler_params=pltpu.CompilerParams(vmem_limit_bytes=110 * 1024 * 1024),
    )(A_x.reshape(S, D), A_wqkv, A_wo, B_x.reshape(S, D), B_wq, B_wk.T, B_wv.T, B_wo)
    return out.reshape(1, S, 2 * D)
```

```python
import functools
import math

import jax
import jax.numpy as jnp
from jax import lax
import jax.experimental.pallas as pl
import jax.experimental.pallas.tpu as pltpu

S = 2048
D = 640
H = 32
DH = 20
QB = 512
T = QB // 128
NQ = S // QB
KC = 128
NK = S // KC
NITEMS = NQ * H
QSCALE = (DH ** -0.5) * math.log2(math.e)
KW = 48
NVG = 80
PNVG = 64
NCH = 2
DBLS = (7, 8)
DOFF = 1
BACK = 3
NBC = 640
KPAD = 3
KOFF = 2
UA = 2
MIDLAG = 8
INFLATE = 1.0 + 2.0 ** -6
LMIN = 2.0 ** -30
ONES2 = 0x3F803F80

f32 = jnp.float32
bf16 = jnp.bfloat16
u32 = jnp.uint32
NT = (((1,), (1,)), ((), ()))
TN = (((0,), (0,)), ((), ()))


def _colbcast(row):
    return jnp.broadcast_to(row, (128, 128)).T


def _steps(nd):
    ns = DH - nd
    dbl = set(((i * ns) // nd + DOFF) % ns for i in range(nd))
    steps = []
    for i in range(ns):
        d0 = sum(len(s) for s in steps)
        steps.append(list(range(d0, d0 + (2 if i in dbl else 1))))
    return steps


def _kernel(xa_h, wqkv_h, woa_h, xb_h, wq_h, wkt_h, wvt_h, wob_h,
            out_h,
            xa, wqkv, woa, xb, wq, wkt, wvt, wob, wtb,
            qta, qtb, ka, kb, vta, vtb, ota, otb, ra, rb, kbc, kca, kcb,
            s0, s1, s2, s3, s4, s5, s6, s7, sx,
            qr0, qr1, qr2, qr3, wa0, wa1, wa2, wa3, wb0, wb1, wb2, wb3, ra1, rb1, ra2, rb2, ra3, rb3, okv,
            part, obuf, tab, isem, osem):
    def cp(i, src, dst):
        return pltpu.make_async_copy(src, dst, isem.at[i])

    def cp_rows(base, src, dst, r):
        rows = pl.ds(r * QB, QB)
        return pltpu.make_async_copy(src.at[rows, :], dst.at[rows, :], isem.at[base + r])

    c_b = [cp(0, wq_h, wq), cp(1, wkt_h, wkt), cp(2, wvt_h, wvt)]
    c_a = cp(3, wqkv_h, wqkv)
    c_wo = [cp(4, woa_h, woa), cp(5, wob_h, wob)]
    for c in c_b:
        c.start()
    cp_rows(6, xb_h, xb, 0).start()

    tab[0] = 0
    tab[1] = 0

    for r in range(1, NQ):
        cp_rows(6, xb_h, xb, r).start()
    c_a.start()
    for r in range(NQ):
        cp_rows(10, xa_h, xa, r).start()
    for c in c_wo:
        c.start()
    okv[...] = jnp.full(okv.shape, 1.0, f32)
    for r_ in (ra2, rb2, ra3, rb3):
        r_[...] = jnp.full(r_.shape, 1.0, f32)

    for c in c_b:
        c.wait()
    zpad = jnp.zeros((4, D), bf16)
    wtb[0:(D + 48) // 2, :] = pltpu.bitcast(
        jnp.concatenate([wkt[...], zpad, wvt[...], zpad, wq[...].T], axis=0), u32)

    def proj_b(r, kabs):
        cp_rows(6, xb_h, xb, r).wait()
        xblk = xb[pl.ds(pl.multiple_of(r * QB, QB), QB), :]
        qv = lax.dot_general(pltpu.bitcast(wtb[0:(D + 48) // 2, :], bf16), xblk, NT,
                             preferred_element_type=f32)
        k = jnp.concatenate([qv[0:24], jnp.zeros((8, QB), f32)], axis=0).T.astype(bf16)
        v = qv[24:48]
        q = qv[48:]
        kabs = jnp.maximum(kabs, jnp.max(jnp.abs(k.astype(f32)).reshape(QB // 8, 8, 32), axis=0))
        lane = lax.broadcasted_iota(jnp.int32, (QB // 2, 32), 1)
        kb[pl.ds(pl.multiple_of(r * (QB // 2), QB // 2), QB // 2), :] = jnp.where(
            lane == DH, jnp.uint32(ONES2), pltpu.bitcast(k, u32))
        rid = lax.broadcasted_iota(jnp.int32, (24, QB), 0)
        vtb[r, 0] = jnp.where(rid == DH, 1.0, v)
        vtb[r, 1] = jnp.where(rid == 0, 1.0, qv[20:44])
        qtb[r] = (q * QSCALE).astype(bf16).astype(f32)
        return kabs

    kabs = lax.fori_loop(0, NQ, proj_b, jnp.zeros((8, 32), f32))
    kabs = jnp.max(kabs, axis=0, keepdims=True) * INFLATE
    kcb[...] = _colbcast(jnp.concatenate([kabs, jnp.zeros((1, 96), f32)], axis=1))[0:32]

    c_a.wait()

    def proj_a(r, kabs):
        xblk = xa[pl.ds(pl.multiple_of(r * QB, QB), QB), :]
        k = jnp.dot(xblk, wqkv[:, D:2 * D], preferred_element_type=f32).astype(bf16)
        kabs = jnp.maximum(kabs, jnp.max(jnp.abs(k.astype(f32)).reshape(QB // 8, 8, D), axis=0))
        ku = pltpu.bitcast(k, u32)
        ku = jnp.concatenate([ku, ku[:, 0:128]], axis=1)
        lane = lax.broadcasted_iota(jnp.int32, (QB // 2, KW), 1)
        for g in range(H // 2):
            ka[g, pl.ds(pl.multiple_of(r * (QB // 2), QB // 2), QB // 2), :] = jnp.where(
                lane == 2 * DH, jnp.uint32(ONES2), ku[:, 2 * DH * g:2 * DH * g + KW])
        nb = NBC // NQ
        kf = pltpu.bitcast(kb[pl.ds(pl.multiple_of((S - NBC) // 2 + r * (nb // 2), 8), nb // 2), :],
                           bf16).astype(f32)
        for d in range(DH):
            kbc[d, pl.ds(pl.multiple_of(r * nb + 8 * KOFF, 8), nb), :] = jnp.broadcast_to(kf[:, d:d + 1], (nb, 128))
        wt = jnp.concatenate([wqkv[:, 0:D].T, wqkv[:, 2 * D:3 * D].T], axis=0)
        qv = lax.dot_general(wt, xblk, NT, preferred_element_type=f32)
        qta[r] = qv[:D] * QSCALE
        vta[r] = qv[D:].reshape(H // 2, 2 * DH, QB)
        return kabs

    def proj_a2(i, kabs):
        for u in range(UA):
            cp_rows(10, xa_h, xa, i * UA + u).wait()
        for u in range(UA):
            kabs = proj_a(i * UA + u, kabs)
        return kabs

    kabs = lax.fori_loop(0, NQ // UA, proj_a2, jnp.zeros((8, D), f32))
    kabs = jnp.max(kabs, axis=0, keepdims=True) * INFLATE
    for g in range(D // 128):
        kca[g * 128:(g + 1) * 128, :] = _colbcast(kabs[:, g * 128:(g + 1) * 128])

    qrs = (qr0, qr1, qr2, qr3)
    was = (wa0, wa1, wa2, wa3)
    wbs = (wb0, wb1, wb2, wb3)
    sbuf = ((s0, s1), (s2, s3), (s4, s5), (s6, s7))
    raw = ((ra, rb), (ra1, rb1), (ra2, rb2), (ra3, rb3))

    def prep(j2, slot, exact):
        par2 = slot & 1
        qi = j2 >> 5
        h = j2 & (H - 1)
        hs = pl.multiple_of((h >> 1) * 2 * DH + 16 * par2, 8)
        r24 = lax.broadcasted_iota(jnp.int32, (24, QB), 0)
        z8 = jnp.zeros((8, QB), f32)
        t = jnp.where((r24 < DH) if par2 == 0 else (r24 >= 4), qta[qi, pl.ds(hs, 24), :], 0.0)
        last = z8
        if not exact:
            nb = -jnp.sum(jnp.abs(t) * jnp.concatenate([kca[pl.ds(hs, 24), :]] * T, axis=1), axis=0, keepdims=True)
            last = jnp.where(lax.broadcasted_iota(jnp.int32, (8, QB), 0) == 0, nb, 0.0)
        w = jnp.concatenate([t, z8, z8, last] if par2 == 0 else [z8, z8, t, last], axis=0)
        was[slot][0:24, :] = pltpu.bitcast(w.astype(bf16), u32)
        q = qtb[qi, pl.ds(hs, 24), :]
        if par2:
            q = jnp.concatenate([q[4:24], q[0:4]], axis=0)
        q = jnp.where(r24 < DH, q, 0.0)
        if not exact:
            nb = -jnp.sum(jnp.abs(q) * jnp.concatenate([kcb[0:24, :]] * T, axis=1), axis=0, keepdims=True)
            nb = nb.astype(bf16).astype(f32)
            q = jnp.where(r24 == DH, nb, q)
            qrs[slot][...] = q
        wbs[slot][...] = pltpu.bitcast(jnp.concatenate([q, jnp.zeros((8, QB), f32)], axis=0).astype(bf16), u32)

    def wload(w, s):
        return pltpu.bitcast(wbs[s][...] if w else was[s][0:24, :], bf16)

    def vslab(w, par, hp, blk, cols):
        if w == 1:
            return vtb[blk, par, :, cols]
        mid = vta[blk, hp, 16:24, cols]
        rid = lax.broadcasted_iota(jnp.int32, mid.shape, 0)
        if par == 0:
            return jnp.concatenate([vta[blk, hp, 0:16, cols], jnp.where(rid == 4, 1.0, mid)], axis=0)
        return jnp.concatenate([jnp.where(rid == 0, 1.0, mid), vta[blk, hp, 24:40, cols]], axis=0)

    def normalize(j, slot, ws=(0, 1)):
        par = slot & 1
        hp = (j & (H - 1)) >> 1
        for w in ws:
            a = raw[slot][w][...]
            den = a[0:1, :] if par else a[DH:DH + 1, :]
            okv[w:w + 1, :] = jnp.where(den >= LMIN, okv[w:w + 1, :], -1.0)
            o = a * (1.0 / den)
            (ota if w == 0 else otb)[hp, par * DH:(par + 1) * DH, :] = o[4:24] if par else o[0:DH]

    def block(j, s0_, do1=True, do2=True, nvg=NVG, extra=(), mid=None):
        nm = S - nvg * 8
        hp = (j & (H - 1)) >> 1
        never = lax.broadcasted_iota(jnp.int32, (8, 128), 0) > (tab[0] + 1000)
        hist = []
        accs = {}
        rounds = [(u, r, l) for u in range(2) for l in range(T) for r in range(0, nvg, NCH)] if do1 else []
        stepsets = [_steps(nd) for nd in (DBLS if do2 else DBLS[:1])]
        s1_ = (s0_ + 2) & 3
        g1 = ((j + 2) & (H - 1)) >> 1

        def vpu_gen():
            for ir, (u, r, l) in enumerate(rounds):
                cols = slice(l * 128, (l + 1) * 128)
                if r == 0:
                    q24 = jnp.where(never[None], hist[-BACK][0][None] if hist else 3.0,
                                    qrs[s1_ + u][:, cols].reshape(3, 8, 128)).reshape(24, 128)
                    qq = [jnp.broadcast_to(q24[d:d + 1], (8, 128)) for d in range(DH + 1)]
                kk = kbc[:, pl.ds(NBC - nvg * 8 + r * 8 + 8 * KOFF, 8 * NCH), :]
                kk = kk.reshape(DH, NCH, 8, 128)
                acc = jnp.broadcast_to(qq[DH][None], (NCH, 8, 128))
                if hist:
                    acc = jnp.where(never[None], hist[-1], acc)
                for st in stepsets[ir % len(stepsets)]:
                    acc = acc + functools.reduce(jnp.add, [kk[d] * qq[d][None] for d in st])
                sbuf[s1_ + u][1][pl.ds(nm + r * 8, 8 * NCH), cols] = acc.reshape(8 * NCH, 128)
                hist.append(acc)
                yield

        def tie(x):
            return jnp.concatenate([jnp.where(never, jnp.max(hist[-1], axis=0), x[:, 0:128]), x[:, 128:]], axis=1)

        def qk(u, w, r0, nr):
            qm = wload(w, s1_ + u)
            kblk = ka[g1, pl.ds(r0 // 2, nr // 2), :] if w == 0 else kb[pl.ds(r0 // 2, nr // 2), :]
            sc = jnp.dot(pltpu.bitcast(kblk, bf16), qm, preferred_element_type=f32)
            if not do2 and (u, w, r0, nr) == qus[-1]:
                for _ in gen:
                    pass
                sc = jnp.concatenate([sc[:nr - 8], tie(sc[nr - 8:])], axis=0)
            sbuf[s1_ + u][w][pl.ds(r0, nr), :] = sc

        def pv(u, w, c):
            p = jnp.exp2(sbuf[s0_ + u][w][pl.ds(c * KC, KC), :])
            v = vslab(w, u, hp, c // T, slice((c % T) * KC, (c % T + 1) * KC))
            d_ = jnp.dot(v, p, preferred_element_type=f32)
            if c > 0:
                accs[w] = accs[w] + d_
            elif u == 1 and do1:
                nv = jnp.concatenate([never] * T, axis=1)
                accs[w] = jnp.where(nv[None], accs[w].reshape(3, 8, QB), d_.reshape(3, 8, QB)).reshape(24, QB)
            else:
                accs[w] = d_
            if c == NK - 1 and not (w == 1 and u == 1):
                raw[s0_ + u][w][...] = accs[w]

        qus = []
        pus = []
        for u in range(2):
            for c in range(NK):
                b0 = ((c * (nm // 16)) // NK) * 16
                b1 = (((c + 1) * (nm // 16)) // NK) * 16
                qus += [(u, 1, b0, b1 - b0), (u, 0, c * KC, KC)]
                pus += [(u, 0, c), (u, 1, c)]
        if not do2:
            qus = qus[0::2] + qus[1::2]
        if mid is not None:
            pus = pus[0::2] + pus[1::2]
        gen = vpu_gen()
        for u in range(2):
            if do1:
                prep((j + 4 + u) & (NITEMS - 1), s0_ + u, False)
            if do2:
                normalize(j - 2 + u, s1_ + u)
        done = 0
        for i in range(4 * NK):
            if mid is not None and i == 2 * NK + MIDLAG:
                mid()
            if do1:
                qk(*qus[i])
            for e in extra[(i * len(extra)) // (4 * NK):((i + 1) * len(extra)) // (4 * NK)]:
                e()
            if do2:
                pv(*pus[i])
            while done < ((i + 1) * len(rounds)) // (4 * NK) and (do2 or i < 4 * NK - 1):
                next(gen)
                done += 1
        if do2:
            a = accs[1]
            raw[s0_ + 1][1][...] = jnp.concatenate([tie(a[0:8]), a[8:]], axis=0) if do1 else a

    def exact_item(j, par):
        prep(j, par, True)
        h = j & (H - 1)
        for w in (0, 1):
            qm = wload(w, par)

            def scores(b, m, w=w, qm=qm):
                rows = pl.ds(pl.multiple_of(b * (QB // 2), QB // 2), QB // 2)
                kblk = ka[h >> 1, rows, :] if w == 0 else kb[rows, :]
                sc = jnp.dot(pltpu.bitcast(kblk, bf16), qm, preferred_element_type=f32)
                sx[pl.ds(pl.multiple_of(b * QB, QB), QB), :] = sc
                return jnp.maximum(m, jnp.max(sc.reshape(QB // 8, 8, QB), axis=0))

            m = lax.fori_loop(0, NQ, scores, jnp.full((8, QB), -jnp.inf, f32))
            m = jnp.max(m, axis=0, keepdims=True)

            def weighted(b, acc, w=w, m=m):
                p = jnp.exp2(sx[pl.ds(pl.multiple_of(b * QB, QB), QB), :] - m)
                return acc + jnp.dot(vslab(w, par, h >> 1, b, slice(None)), p, preferred_element_type=f32)

            raw[2 + par][w][...] = lax.fori_loop(0, NQ, weighted, jnp.zeros((24, QB), f32))
        normalize(j, 2 + par)

    def out_copy(qi, w):
        slot = qi & 1
        return pltpu.make_async_copy(obuf.at[2 * slot + w], out_h.at[pl.ds(qi * QB, QB), w * D:(w + 1) * D],
                                     osem.at[2 * slot + w])

    def out_proj(qi):
        slot = qi & 1

        @pl.when(qi >= 2)
        def _():
            out_copy(qi - 2, 0).wait()
            out_copy(qi - 2, 1).wait()
        normalize(jnp.int32(H - 2), 2)
        normalize(jnp.int32(H - 1), 3)
        oa = ota[...].reshape(D, QB).astype(bf16)
        obuf[2 * slot] = lax.dot_general(oa, woa[...], TN, preferred_element_type=f32).astype(bf16)
        out_copy(qi, 0).start()
        ob = otb[...].reshape(D, QB).astype(bf16)
        obuf[2 * slot + 1] = lax.dot_general(ob, wob[...], TN, preferred_element_type=f32).astype(bf16)
        out_copy(qi, 1).start()

    def final_block():
        qi = NQ - 1
        kp = 512
        out_copy(qi - 2, 0).wait()
        out_copy(qi - 2, 1).wait()
        lhs = {}

        def unit(w, m, n):
            if (w, m) not in lhs:
                o = (ota if w == 0 else otb)[0:13, :, m * 128:(m + 1) * 128].reshape(13 * 2 * DH, 128)[0:kp]
                lhs[w, m] = o.T.astype(bf16)
            part[w, m * 128:(m + 1) * 128, n * 128:(n + 1) * 128] = jnp.dot(
                lhs[w, m], (woa if w == 0 else wob)[0:kp, n * 128:(n + 1) * 128], preferred_element_type=f32)

        extra = [functools.partial(unit, w, m, n) for w in (0, 1) for m in range(T) for n in range(D // 128)]

        def finish(w):
            normalize(jnp.int32(H - 2), 2, (w,))
            normalize(jnp.int32(H - 1), 3, (w,))
            o = (ota if w == 0 else otb)[12:16].reshape(4 * 2 * DH, QB)[kp - 12 * 2 * DH:].astype(bf16)
            rest = lax.dot_general(o, (woa if w == 0 else wob)[kp:, :], TN, preferred_element_type=f32)
            obuf[2 * (qi & 1) + w] = (part[w] + rest).astype(bf16)
            out_copy(qi, w).start()

        block(jnp.int32(NITEMS - 2), 2, do1=False, extra=extra, mid=functools.partial(finish, 0))
        finish(1)

    prep(jnp.int32(0), 0, False)
    prep(jnp.int32(1), 1, False)
    block(jnp.int32(-2), 2, do2=False, nvg=PNVG)

    def one_pass(p, carry):
        @pl.when(tab[1] == 0)
        def _():
            def body(i, c2):
                j = 4 * i

                @pl.when(p == 0)
                def _():
                    block(j, 0)

                @pl.when((p == 0) & (j + 2 < NITEMS - 2))
                def _():
                    block(j + 2, 2)

                @pl.when((p != 0) | ((j & (H - 1)) == H - 4))
                def _():
                    @pl.when((p == 0) & (j + 2 == NITEMS - 2))
                    def _():
                        final_block()

                    @pl.when(p != 0)
                    def _():
                        def pair(u, c3):
                            exact_item(j + 2 * u, 0)
                            exact_item(j + 2 * u + 1, 1)
                            return c3
                        lax.fori_loop(0, 2, pair, 0)

                    @pl.when(((j & (H - 1)) == H - 4) & ((p != 0) | (j + 2 != NITEMS - 2)))
                    def _():
                        out_proj(j >> 5)
                return c2

            lax.fori_loop(0, NITEMS // 4, body, 0)
            tab[1] = jnp.where(jnp.min(okv[...]) > 0.5, 1, 0)
            for qi in (NQ - 2, NQ - 1):
                for w in (0, 1):
                    out_copy(qi, w).wait()
        return carry

    for c in c_wo:
        c.wait()
    lax.fori_loop(0, 2, one_pass, 0)


@jax.jit
def pallas_concat_heads__softmax_full_mha__grouped_kv_mqa__prompt_kernel(
        A_x, A_wqkv, A_wo, B_x, B_wq, B_wk, B_wv, B_wo):
    V = pltpu.VMEM
    scratch = [
        V((S, D), bf16), V((D, 3 * D), bf16), V((D, D), bf16), V((S, D), bf16), V((D, D), bf16),
        V((DH, D), bf16), V((DH, D), bf16), V((D, D), bf16), V(((D + 64) // 2, D), u32),
        V((NQ, D, QB), f32), V((NQ, D, QB), f32), V((H // 2, S // 2, KW), u32), V((S // 2, 32), u32),
        V((NQ, H // 2, 2 * DH, QB), f32), V((NQ, 2, 24, QB), f32),
        V((H // 2, 2 * DH, QB), f32), V((H // 2, 2 * DH, QB), f32), V((24, QB), f32), V((24, QB), f32),
        V((DH, NBC + 8 * KPAD, 128), f32), V((D, 128), f32), V((32, 128), f32),
    ] + [V((S, QB), f32)] * 9 + [V((24, QB), f32)] * 4 + [V((32, QB), u32)] * 4 + [
        V((16, QB), u32)] * 4 + [V((24, QB), f32)] * 6 + [
        V((8, QB), f32),
        V((2, QB, D), f32), V((4, QB, D), bf16), pltpu.SMEM((2,), jnp.int32),
        pltpu.SemaphoreType.DMA((14,)), pltpu.SemaphoreType.DMA((4,)),
    ]
    out = pl.pallas_call(
        _kernel,
        out_shape=jax.ShapeDtypeStruct((S, 2 * D), bf16),
        in_specs=[pl.BlockSpec(memory_space=pl.ANY)] * 8,
        out_specs=pl.BlockSpec(memory_space=pl.ANY),
        scratch_shapes=scratch,
        compiler_params=pltpu.CompilerParams(vmem_limit_bytes=110 * 1024 * 1024),
    )(A_x.reshape(S, D), A_wqkv, A_wo, B_x.reshape(S, D), B_wq, B_wk.T, B_wv.T, B_wo)
    return out.reshape(1, S, 2 * D)
```

```python
import functools
import math

import jax
import jax.numpy as jnp
from jax import lax
import jax.experimental.pallas as pl
import jax.experimental.pallas.tpu as pltpu

S = 2048
D = 640
H = 32
DH = 20
QB = 512
T = QB // 128
NQ = S // QB
KC = 128
NK = S // KC
NITEMS = NQ * H
QSCALE = (DH ** -0.5) * math.log2(math.e)
KW = 48
NVG = 80
PNVG = 72
NCH = 2
DBLS = (7, 8)
DOFF = 1
BACK = 3
NBC = 640
KPAD = 3
KOFF = 2
UA = 2
MIDLAG = 8
INFLATE = 1.0 + 2.0 ** -6
LMIN = 2.0 ** -30
ONES2 = 0x3F803F80

f32 = jnp.float32
bf16 = jnp.bfloat16
u32 = jnp.uint32
NT = (((1,), (1,)), ((), ()))
TN = (((0,), (0,)), ((), ()))


def _colbcast(row):
    return jnp.broadcast_to(row, (128, 128)).T


def _steps(nd):
    ns = DH - nd
    dbl = set(((i * ns) // nd + DOFF) % ns for i in range(nd))
    steps = []
    for i in range(ns):
        d0 = sum(len(s) for s in steps)
        steps.append(list(range(d0, d0 + (2 if i in dbl else 1))))
    return steps


def _kernel(xa_h, wqkv_h, woa_h, xb_h, wq_h, wkt_h, wvt_h, wob_h,
            out_h,
            xa, wqkv, woa, xb, wq, wkt, wvt, wob, wtb,
            qta, qtb, ka, kb, vta, vtb, ota, otb, ra, rb, kbc, kca, kcb,
            s0, s1, s2, s3, s4, s5, s6, s7, sx,
            qr0, qr1, qr2, qr3, wa0, wa1, wa2, wa3, wb0, wb1, wb2, wb3, ra1, rb1, ra2, rb2, ra3, rb3, okv,
            part, obuf, tab, isem, osem):
    def cp(i, src, dst):
        return pltpu.make_async_copy(src, dst, isem.at[i])

    def cp_rows(base, src, dst, r):
        rows = pl.ds(r * QB, QB)
        return pltpu.make_async_copy(src.at[rows, :], dst.at[rows, :], isem.at[base + r])

    c_b = [cp(0, wq_h, wq), cp(1, wkt_h, wkt), cp(2, wvt_h, wvt)]
    c_a = cp(3, wqkv_h, wqkv)
    c_wo = [cp(4, woa_h, woa), cp(5, wob_h, wob)]
    for c in c_b:
        c.start()
    cp_rows(6, xb_h, xb, 0).start()

    tab[0] = 0
    tab[1] = 0

    for r in range(1, NQ):
        cp_rows(6, xb_h, xb, r).start()
    c_a.start()
    for r in range(NQ):
        cp_rows(10, xa_h, xa, r).start()
    for c in c_wo:
        c.start()
    okv[...] = jnp.full(okv.shape, 1.0, f32)
    for r_ in (ra2, rb2, ra3, rb3):
        r_[...] = jnp.full(r_.shape, 1.0, f32)

    for c in c_b:
        c.wait()
    zpad = jnp.zeros((4, D), bf16)
    wtb[0:(D + 48) // 2, :] = pltpu.bitcast(
        jnp.concatenate([wkt[...], zpad, wvt[...], zpad, wq[...].T], axis=0), u32)

    def proj_b(r, kabs):
        cp_rows(6, xb_h, xb, r).wait()
        xblk = xb[pl.ds(pl.multiple_of(r * QB, QB), QB), :]
        qv = lax.dot_general(pltpu.bitcast(wtb[0:(D + 48) // 2, :], bf16), xblk, NT,
                             preferred_element_type=f32)
        k = jnp.concatenate([qv[0:24], jnp.zeros((8, QB), f32)], axis=0).T.astype(bf16)
        v = qv[24:48]
        q = qv[48:]
        kabs = jnp.maximum(kabs, jnp.max(jnp.abs(k.astype(f32)).reshape(QB // 8, 8, 32), axis=0))
        lane = lax.broadcasted_iota(jnp.int32, (QB // 2, 32), 1)
        kb[pl.ds(pl.multiple_of(r * (QB // 2), QB // 2), QB // 2), :] = jnp.where(
            lane == DH, jnp.uint32(ONES2), pltpu.bitcast(k, u32))
        rid = lax.broadcasted_iota(jnp.int32, (24, QB), 0)
        vtb[r, 0] = jnp.where(rid == DH, 1.0, v)
        vtb[r, 1] = jnp.where(rid == 0, 1.0, qv[20:44])
        qtb[r] = (q * QSCALE).astype(bf16).astype(f32)
        return kabs

    kabs = lax.fori_loop(0, NQ, proj_b, jnp.zeros((8, 32), f32))
    kabs = jnp.max(kabs, axis=0, keepdims=True) * INFLATE
    kcb[...] = _colbcast(jnp.concatenate([kabs, jnp.zeros((1, 96), f32)], axis=1))[0:32]

    c_a.wait()

    def proj_a(r, kabs):
        xblk = xa[pl.ds(pl.multiple_of(r * QB, QB), QB), :]
        k = jnp.dot(xblk, wqkv[:, D:2 * D], preferred_element_type=f32).astype(bf16)
        kabs = jnp.maximum(kabs, jnp.max(jnp.abs(k.astype(f32)).reshape(QB // 8, 8, D), axis=0))
        ku = pltpu.bitcast(k, u32)
        ku = jnp.concatenate([ku, ku[:, 0:128]], axis=1)
        lane = lax.broadcasted_iota(jnp.int32, (QB // 2, KW), 1)
        for g in range(H // 2):
            ka[g, pl.ds(pl.multiple_of(r * (QB // 2), QB // 2), QB // 2), :] = jnp.where(
                lane == 2 * DH, jnp.uint32(ONES2), ku[:, 2 * DH * g:2 * DH * g + KW])
        nb = NBC // NQ
        kf = pltpu.bitcast(kb[pl.ds(pl.multiple_of((S - NBC) // 2 + r * (nb // 2), 8), nb // 2), :],
                           bf16).astype(f32)
        for d in range(DH):
            kbc[d, pl.ds(pl.multiple_of(r * nb + 8 * KOFF, 8), nb), :] = jnp.broadcast_to(kf[:, d:d + 1], (nb, 128))
        wt = jnp.concatenate([wqkv[:, 0:D].T, wqkv[:, 2 * D:3 * D].T], axis=0)
        qv = lax.dot_general(wt, xblk, NT, preferred_element_type=f32)
        qta[r] = qv[:D] * QSCALE
        vta[r] = qv[D:].reshape(H // 2, 2 * DH, QB)
        return kabs

    def proj_a2(i, kabs):
        for u in range(UA):
            cp_rows(10, xa_h, xa, i * UA + u).wait()
        for u in range(UA):
            kabs = proj_a(i * UA + u, kabs)
        return kabs

    kabs = lax.fori_loop(0, NQ // UA, proj_a2, jnp.zeros((8, D), f32))
    kabs = jnp.max(kabs, axis=0, keepdims=True) * INFLATE
    for g in range(D // 128):
        kca[g * 128:(g + 1) * 128, :] = _colbcast(kabs[:, g * 128:(g + 1) * 128])

    qrs = (qr0, qr1, qr2, qr3)
    was = (wa0, wa1, wa2, wa3)
    wbs = (wb0, wb1, wb2, wb3)
    sbuf = ((s0, s1), (s2, s3), (s4, s5), (s6, s7))
    raw = ((ra, rb), (ra1, rb1), (ra2, rb2), (ra3, rb3))

    def prep(j2, slot, exact):
        par2 = slot & 1
        qi = j2 >> 5
        h = j2 & (H - 1)
        hs = pl.multiple_of((h >> 1) * 2 * DH + 16 * par2, 8)
        r24 = lax.broadcasted_iota(jnp.int32, (24, QB), 0)
        z8 = jnp.zeros((8, QB), f32)
        t = jnp.where((r24 < DH) if par2 == 0 else (r24 >= 4), qta[qi, pl.ds(hs, 24), :], 0.0)
        last = z8
        if not exact:
            nb = -jnp.sum(jnp.abs(t) * jnp.concatenate([kca[pl.ds(hs, 24), :]] * T, axis=1), axis=0, keepdims=True)
            last = jnp.where(lax.broadcasted_iota(jnp.int32, (8, QB), 0) == 0, nb, 0.0)
        w = jnp.concatenate([t, z8, z8, last] if par2 == 0 else [z8, z8, t, last], axis=0)
        was[slot][0:24, :] = pltpu.bitcast(w.astype(bf16), u32)
        q = qtb[qi, pl.ds(hs, 24), :]
        if par2:
            q = jnp.concatenate([q[4:24], q[0:4]], axis=0)
        q = jnp.where(r24 < DH, q, 0.0)
        if not exact:
            nb = -jnp.sum(jnp.abs(q) * jnp.concatenate([kcb[0:24, :]] * T, axis=1), axis=0, keepdims=True)
            nb = nb.astype(bf16).astype(f32)
            q = jnp.where(r24 == DH, nb, q)
            qrs[slot][...] = q
        wbs[slot][...] = pltpu.bitcast(jnp.concatenate([q, jnp.zeros((8, QB), f32)], axis=0).astype(bf16), u32)

    def wload(w, s):
        return pltpu.bitcast(wbs[s][...] if w else was[s][0:24, :], bf16)

    def vslab(w, par, hp, blk, cols):
        if w == 1:
            return vtb[blk, par, :, cols]
        mid = vta[blk, hp, 16:24, cols]
        rid = lax.broadcasted_iota(jnp.int32, mid.shape, 0)
        if par == 0:
            return jnp.concatenate([vta[blk, hp, 0:16, cols], jnp.where(rid == 4, 1.0, mid)], axis=0)
        return jnp.concatenate([jnp.where(rid == 0, 1.0, mid), vta[blk, hp, 24:40, cols]], axis=0)

    def normalize(j, slot, ws=(0, 1)):
        par = slot & 1
        hp = (j & (H - 1)) >> 1
        for w in ws:
            a = raw[slot][w][...]
            den = a[0:1, :] if par else a[DH:DH + 1, :]
            okv[w:w + 1, :] = jnp.where(den >= LMIN, okv[w:w + 1, :], -1.0)
            o = a * (1.0 / den)
            (ota if w == 0 else otb)[hp, par * DH:(par + 1) * DH, :] = o[4:24] if par else o[0:DH]

    def block(j, s0_, do1=True, do2=True, nvg=NVG, extra=(), mid=None):
        nm = S - nvg * 8
        hp = (j & (H - 1)) >> 1
        never = lax.broadcasted_iota(jnp.int32, (8, 128), 0) > (tab[0] + 1000)
        hist = []
        accs = {}
        rounds = [(u, r, l) for u in range(2) for l in range(T) for r in range(0, nvg, NCH)] if do1 else []
        stepsets = [_steps(nd) for nd in (DBLS if do2 else DBLS[1:])]
        s1_ = (s0_ + 2) & 3
        g1 = ((j + 2) & (H - 1)) >> 1

        def vpu_gen():
            for ir, (u, r, l) in enumerate(rounds):
                cols = slice(l * 128, (l + 1) * 128)
                if r == 0:
                    q24 = jnp.where(never[None], hist[-BACK][0][None] if hist else 3.0,
                                    qrs[s1_ + u][:, cols].reshape(3, 8, 128)).reshape(24, 128)
                    qq = [jnp.broadcast_to(q24[d:d + 1], (8, 128)) for d in range(DH + 1)]
                kk = kbc[:, pl.ds(NBC - nvg * 8 + r * 8 + 8 * KOFF, 8 * NCH), :]
                kk = kk.reshape(DH, NCH, 8, 128)
                acc = jnp.broadcast_to(qq[DH][None], (NCH, 8, 128))
                if hist:
                    acc = jnp.where(never[None], hist[-1], acc)
                for st in stepsets[ir % len(stepsets)]:
                    acc = acc + functools.reduce(jnp.add, [kk[d] * qq[d][None] for d in st])
                sbuf[s1_ + u][1][pl.ds(nm + r * 8, 8 * NCH), cols] = acc.reshape(8 * NCH, 128)
                hist.append(acc)
                yield

        def tie(x):
            return jnp.concatenate([jnp.where(never, jnp.max(hist[-1], axis=0), x[:, 0:128]), x[:, 128:]], axis=1)

        def qk(u, w, r0, nr):
            qm = wload(w, s1_ + u)
            kblk = ka[g1, pl.ds(r0 // 2, nr // 2), :] if w == 0 else kb[pl.ds(r0 // 2, nr // 2), :]
            sc = jnp.dot(pltpu.bitcast(kblk, bf16), qm, preferred_element_type=f32)
            if not do2 and (u, w, r0, nr) == qus[-1]:
                for _ in gen:
                    pass
                sc = jnp.concatenate([sc[:nr - 8], tie(sc[nr - 8:])], axis=0)
            sbuf[s1_ + u][w][pl.ds(r0, nr), :] = sc

        def pv(u, w, c):
            p = jnp.exp2(sbuf[s0_ + u][w][pl.ds(c * KC, KC), :])
            v = vslab(w, u, hp, c // T, slice((c % T) * KC, (c % T + 1) * KC))
            d_ = jnp.dot(v, p, preferred_element_type=f32)
            if c > 0:
                accs[w] = accs[w] + d_
            elif u == 1 and do1:
                prev = accs[w].reshape(3, 8, QB)
                nv = jnp.concatenate([never] * T, axis=1)
                accs[w] = jnp.where(nv[None], prev, d_.reshape(3, 8, QB)).reshape(24, QB)
            else:
                accs[w] = d_
            if c == NK - 1 and not (w == 1 and u == 1):
                raw[s0_ + u][w][...] = accs[w]

        qus = []
        pus = []
        for u in range(2):
            for c in range(NK):
                b0 = ((c * (nm // 16)) // NK) * 16
                b1 = (((c + 1) * (nm // 16)) // NK) * 16
                qus += [(u, 1, b0, b1 - b0), (u, 0, c * KC, KC)]
                pus += [(u, 0, c), (u, 1, c)]
        if not do2:
            qus = qus[0::2] + qus[1::2]
        if mid is not None:
            pus = pus[0::2] + pus[1::2]
        gen = vpu_gen()
        side = []
        for u in range(2):
            if do1:
                side.append(functools.partial(prep, (j + 4 + u) & (NITEMS - 1), s0_ + u, False))
            if do2:
                side.append(functools.partial(normalize, j - 2 + u, s1_ + u))
        for f in side:
            f()
        done = 0
        for i in range(4 * NK):
            if mid is not None and i == 2 * NK + MIDLAG:
                mid()
            if do1:
                qk(*qus[i])
            for e in extra[(i * len(extra)) // (4 * NK):((i + 1) * len(extra)) // (4 * NK)]:
                e()
            if do2:
                pv(*pus[i])
            while done < ((i + 1) * len(rounds)) // (4 * NK) and (do2 or i < 4 * NK - 1):
                next(gen)
                done += 1
        if do2:
            a = accs[1]
            raw[s0_ + 1][1][...] = jnp.concatenate([tie(a[0:8]), a[8:]], axis=0) if do1 else a

    def exact_item(j, par):
        prep(j, par, True)
        h = j & (H - 1)
        for w in (0, 1):
            qm = wload(w, par)

            def scores(b, m, w=w, qm=qm):
                rows = pl.ds(pl.multiple_of(b * (QB // 2), QB // 2), QB // 2)
                kblk = ka[h >> 1, rows, :] if w == 0 else kb[rows, :]
                sc = jnp.dot(pltpu.bitcast(kblk, bf16), qm, preferred_element_type=f32)
                sx[pl.ds(pl.multiple_of(b * QB, QB), QB), :] = sc
                return jnp.maximum(m, jnp.max(sc.reshape(QB // 8, 8, QB), axis=0))

            m = lax.fori_loop(0, NQ, scores, jnp.full((8, QB), -jnp.inf, f32))
            m = jnp.max(m, axis=0, keepdims=True)

            def weighted(b, acc, w=w, m=m):
                p = jnp.exp2(sx[pl.ds(pl.multiple_of(b * QB, QB), QB), :] - m)
                return acc + jnp.dot(vslab(w, par, h >> 1, b, slice(None)), p, preferred_element_type=f32)

            raw[2 + par][w][...] = lax.fori_loop(0, NQ, weighted, jnp.zeros((24, QB), f32))
        normalize(j, 2 + par)

    def out_copy(qi, w):
        slot = qi & 1
        return pltpu.make_async_copy(obuf.at[2 * slot + w], out_h.at[pl.ds(qi * QB, QB), w * D:(w + 1) * D],
                                     osem.at[2 * slot + w])

    def out_proj(qi):
        slot = qi & 1

        @pl.when(qi >= 2)
        def _():
            out_copy(qi - 2, 0).wait()
            out_copy(qi - 2, 1).wait()
        normalize(jnp.int32(H - 2), 2)
        normalize(jnp.int32(H - 1), 3)
        oa = ota[...].reshape(D, QB).astype(bf16)
        obuf[2 * slot] = lax.dot_general(oa, woa[...], TN, preferred_element_type=f32).astype(bf16)
        out_copy(qi, 0).start()
        ob = otb[...].reshape(D, QB).astype(bf16)
        obuf[2 * slot + 1] = lax.dot_general(ob, wob[...], TN, preferred_element_type=f32).astype(bf16)
        out_copy(qi, 1).start()

    def final_block():
        qi = NQ - 1
        kp = 512
        out_copy(qi - 2, 0).wait()
        out_copy(qi - 2, 1).wait()
        lhs = {}

        def unit(w, m, n):
            if (w, m) not in lhs:
                o = (ota if w == 0 else otb)[0:13, :, m * 128:(m + 1) * 128].reshape(13 * 2 * DH, 128)[0:kp]
                lhs[w, m] = o.T.astype(bf16)
            part[w, m * 128:(m + 1) * 128, n * 128:(n + 1) * 128] = jnp.dot(
                lhs[w, m], (woa if w == 0 else wob)[0:kp, n * 128:(n + 1) * 128], preferred_element_type=f32)

        extra = [functools.partial(unit, w, m, n) for w in (0, 1) for m in range(T) for n in range(D // 128)]

        def finish(w):
            normalize(jnp.int32(H - 2), 2, (w,))
            normalize(jnp.int32(H - 1), 3, (w,))
            o = (ota if w == 0 else otb)[12:16].reshape(4 * 2 * DH, QB)[kp - 12 * 2 * DH:].astype(bf16)
            for m in range(2):
                rows = slice(m * QB // 2, (m + 1) * QB // 2)
                rest = lax.dot_general(o[:, rows], (woa if w == 0 else wob)[kp:, :], TN, preferred_element_type=f32)
                obuf[2 * (qi & 1) + w, rows, :] = (part[w, rows, :] + rest).astype(bf16)
            out_copy(qi, w).start()

        block(jnp.int32(NITEMS - 2), 2, do1=False, extra=extra, mid=functools.partial(finish, 0))
        finish(1)

    prep(jnp.int32(0), 0, False)
    prep(jnp.int32(1), 1, False)
    block(jnp.int32(-2), 2, do2=False, nvg=PNVG)

    def one_pass(p, carry):
        @pl.when(tab[1] == 0)
        def _():
            def body(i, c2):
                j = 4 * i

                @pl.when(p == 0)
                def _():
                    block(j, 0)

                @pl.when((p == 0) & (j + 2 < NITEMS - 2))
                def _():
                    block(j + 2, 2)

                @pl.when((p != 0) | ((j & (H - 1)) == H - 4))
                def _():
                    @pl.when((p == 0) & (j + 2 == NITEMS - 2))
                    def _():
                        final_block()

                    @pl.when(p != 0)
                    def _():
                        def pair(u, c3):
                            exact_item(j + 2 * u, 0)
                            exact_item(j + 2 * u + 1, 1)
                            return c3
                        lax.fori_loop(0, 2, pair, 0)

                    @pl.when(((j & (H - 1)) == H - 4) & ((p != 0) | (j + 2 != NITEMS - 2)))
                    def _():
                        out_proj(j >> 5)
                return c2

            lax.fori_loop(0, NITEMS // 4, body, 0)
            tab[1] = jnp.where(jnp.min(okv[...]) > 0.5, 1, 0)
            for qi in (NQ - 2, NQ - 1):
                for w in (0, 1):
                    out_copy(qi, w).wait()
        return carry

    for c in c_wo:
        c.wait()
    lax.fori_loop(0, 2, one_pass, 0)


@jax.jit
def pallas_concat_heads__softmax_full_mha__grouped_kv_mqa__prompt_kernel(
        A_x, A_wqkv, A_wo, B_x, B_wq, B_wk, B_wv, B_wo):
    V = pltpu.VMEM
    scratch = [
        V((S, D), bf16), V((D, 3 * D), bf16), V((D, D), bf16), V((S, D), bf16), V((D, D), bf16),
        V((DH, D), bf16), V((DH, D), bf16), V((D, D), bf16), V(((D + 64) // 2, D), u32),
        V((NQ, D, QB), f32), V((NQ, D, QB), f32), V((H // 2, S // 2, KW), u32), V((S // 2, 32), u32),
        V((NQ, H // 2, 2 * DH, QB), f32), V((NQ, 2, 24, QB), f32),
        V((H // 2, 2 * DH, QB), f32), V((H // 2, 2 * DH, QB), f32), V((24, QB), f32), V((24, QB), f32),
        V((DH, NBC + 8 * KPAD, 128), f32), V((D, 128), f32), V((32, 128), f32),
    ] + [V((S, QB), f32)] * 9 + [V((24, QB), f32)] * 4 + [V((32, QB), u32)] * 4 + [
        V((16, QB), u32)] * 4 + [V((24, QB), f32)] * 6 + [
        V((8, QB), f32),
        V((2, QB, D), f32), V((4, QB, D), bf16), pltpu.SMEM((2,), jnp.int32),
        pltpu.SemaphoreType.DMA((14,)), pltpu.SemaphoreType.DMA((4,)),
    ]
    out = pl.pallas_call(
        _kernel,
        out_shape=jax.ShapeDtypeStruct((S, 2 * D), bf16),
        in_specs=[pl.BlockSpec(memory_space=pl.ANY)] * 8,
        out_specs=pl.BlockSpec(memory_space=pl.ANY),
        scratch_shapes=scratch,
        compiler_params=pltpu.CompilerParams(vmem_limit_bytes=110 * 1024 * 1024),
    )(A_x.reshape(S, D), A_wqkv, A_wo, B_x.reshape(S, D), B_wq, B_wk.T, B_wv.T, B_wo)
    return out.reshape(1, S, 2 * D)
```
